```python
import jax
import jax.numpy as jnp

def _softmax(x, axis=-1):
    return jax.nn.softmax(x, axis=axis)

def _gelu(x):
    return jax.nn.gelu(x, approximate=True)

def _silu(x):
    return jax.nn.silu(x)

def _sigmoid(x):
    return jax.nn.sigmoid(x)

def _layernorm(x, axis=-1, eps=1e-05):
    m = jnp.mean(x, axis=axis, keepdims=True)
    v = jnp.var(x, axis=axis, keepdims=True)
    return (x - m) / jnp.sqrt(v + eps)

def _scatter_add(tgt, idx, src, axis=0):
    return tgt.at[idx].add(src)

def _segment_sum(src, seg, n):
    return jax.ops.segment_sum(src, seg, n)

class _Rng:

    def __init__(self, key):
        self._k = key

    def _next(self):
        self._k, sub = jax.random.split(self._k)
        return sub

    def normal(self, shape):
        return jax.random.normal(self._next(), shape, dtype=jnp.bfloat16)

    def randint(self, lo, hi, shape):
        return jax.random.randint(self._next(), shape, lo, hi, dtype=jnp.int32)

    def uniform(self, shape, lo=0.0, hi=1.0):
        return jax.random.uniform(self._next(), shape, jnp.bfloat16, lo, hi)

    def permutation(self, n):
        return jax.random.permutation(self._next(), n)
kernel_name = 'adaLN_cond__sliding_local_dilated__swiglu_ffn__prompt'

def setup_inputs():
    _rng = _Rng(jax.random.key(int.from_bytes(__import__("os").urandom(4), "little")))
    _w = lambda a: (lambda t: t.astype(jnp.bfloat16) if jnp.issubdtype(t.dtype, jnp.floating) else t)(jnp.asarray(a))

    def _A_setup():
        B, S, D = (1, 2048, 1024)
        return {'x': _w((lambda *s: _rng.normal(s) * 0.05)(B, S, D)), 'wqkv': _w((lambda *s: _rng.normal(s) * 0.05)(D, 3 * D)), 'wo': _w((lambda *s: _rng.normal(s) * 0.05)(D, D))}
    _A_in = _A_setup()

    def _B_setup():
        B, S, D, F = (1, 2048, 1024, 3584)
        return {'x': _w((lambda *s: _rng.normal(s) * 0.05)(B, S, D)), 'w_gate': _w((lambda *s: _rng.normal(s) * 0.05)(D, F)), 'w_up': _w((lambda *s: _rng.normal(s) * 0.05)(D, F)), 'w_down': _w((lambda *s: _rng.normal(s) * 0.05)(F, D))}
    _B_in = _B_setup()
    return {'A_x': _A_in['x'], 'A_wqkv': _A_in['wqkv'], 'A_wo': _A_in['wo'], 'B_x': _B_in['x'], 'B_w_gate': _B_in['w_gate'], 'B_w_up': _B_in['w_up'], 'B_w_down': _B_in['w_down'], 'c': _w((lambda *s: _rng.normal(s) * 0.05)(1, 1024)), 'w_mod': _w((lambda *s: _rng.normal(s) * 0.05)(1024, 6 * 1024) * 1024 ** (-0.5))}

def reference(A_x, A_wqkv, A_wo, B_x, B_w_gate, B_w_up, B_w_down, c, w_mod):

    def _A_ref(x, wqkv, wo):
        B, S, D = x.shape
        H = 32
        Dh = D // H
        W, dil = (8, 2)
        qkv = (lambda x, *d: x.transpose(*d))((x @ wqkv).reshape(B, S, 3, H, Dh), 2, 0, 3, 1, 4)
        q, k, v = (qkv[0], qkv[1], qkv[2])
        scale = Dh ** (-0.5)
        pos = jnp.arange(S)
        off = jnp.arange(W) * dil
        idx = pos[:, None] - off[None, :]
        mask = idx >= 0
        idx_c = jnp.where(mask, idx, 0).reshape(-1)
        kg = k[:, :, idx_c, :].reshape(B, H, S, W, Dh)
        vg = v[:, :, idx_c, :].reshape(B, H, S, W, Dh)
        logits = jnp.einsum('bhsd,bhswd->bhsw', q, kg) * scale
        logits = jnp.where(mask[None, None, :, :], logits, -1000000000.0)
        attn = _softmax(logits, axis=-1)
        o = jnp.einsum('bhsw,bhswd->bhsd', attn, vg)
        return (lambda x, *d: x.transpose(*d))(o, 0, 2, 1, 3).reshape(B, S, D) @ wo

    def _B_ref(x, w_gate, w_up, w_down):
        g = _silu(x @ w_gate)
        u = x @ w_up
        return g * u @ w_down
    x = A_x
    mod = (_silu(c) @ w_mod).reshape(c.shape[0], 6, 1, -1)
    sa, ca, ga, sb, cb, gb = (mod[:, 0].copy(), mod[:, 1].copy(), mod[:, 2].copy(), mod[:, 3].copy(), mod[:, 4].copy(), mod[:, 5].copy())
    h = _layernorm(x, axis=-1) * (1 + ca) + sa
    x = x + ga * _A_ref(h, A_wqkv, A_wo)
    h = _layernorm(x, axis=-1) * (1 + cb) + sb
    x = x + gb * _B_ref(h, B_w_gate, B_w_up, B_w_down)
    return x
```

```python
import jax
import jax.numpy as jnp
from jax import lax
from jax.experimental import pallas as pl
from jax.experimental.pallas import tpu as pltpu

S, D, F = 2048, 1024, 3584
H, DH, WIN, DIL = 32, 32, 8, 2
TM = 512
NT = S // TM
FC = 512
NF = F // FC
NC = 256
HALO = 16
AR = 16
NG = D // 128
ATT_PER_F = -(-(TM // AR) // NF)
EPS = 1e-5
F32, BF16 = jnp.float32, jnp.bfloat16


def _layernorm(x):
    m = jnp.mean(x, axis=-1, keepdims=True)
    xc = x - m
    v = jnp.mean(xc * xc, axis=-1, keepdims=True)
    return xc * lax.rsqrt(v + EPS)


def _permute_columns(w_ref):
    w32 = w_ref.bitcast(jnp.uint32)
    rows = 16
    lane = lax.broadcasted_iota(jnp.int32, (rows, 128), 1)

    def body(i, carry):
        r = pl.multiple_of(i * rows, rows)
        cols = [w32[pl.ds(r, rows), g * 128:(g + 1) * 128] for g in range(NG)]
        for b in range(3):
            sh = 2 << b
            low = (lane & sh) == 0
            for g in range(NG):
                if g & (1 << b):
                    continue
                lo, hi = cols[g], cols[g | (1 << b)]
                cols[g] = jnp.where(low, lo, pltpu.roll(hi, sh, 1))
                cols[g | (1 << b)] = jnp.where(low, pltpu.roll(lo, 128 - sh, 1), hi)
        for g in range(NG):
            w32[pl.ds(r, rows), g * 128:(g + 1) * 128] = cols[g]
        return carry

    lax.fori_loop(0, D // 2 // rows, body, 0)


def _permute_rows(src_ref, dst_ref):
    s32 = src_ref.bitcast(jnp.uint32)
    d32 = dst_ref.bitcast(jnp.uint32)
    for g in range(NG):
        for j in range(8):
            for m in range(8):
                d32[j * 64 + m * 8:j * 64 + m * 8 + 8, g * 128:(g + 1) * 128] = (
                    s32[g, pl.ds(m * 8 + j, 8, stride=64), :])


def _attention_block(r, pos0, q_s, k_s, v_s, o_s):
    lane = lax.broadcasted_iota(jnp.int32, (AR, 128), 1)
    pos = lax.broadcasted_iota(jnp.int32, (AR, 128), 0) + (pos0 + r)
    even1 = (lane & 1) == 0
    even16 = (lane & 16) == 0
    q = [q_s[g, pl.ds(r, AR), :] for g in range(NG)]
    logits = []
    for w in range(WIN):
        start = r + (HALO - DIL * w)
        acc = q[0] * k_s[0, pl.ds(start, AR), :]
        for g in range(1, NG):
            acc = acc + q[g] * k_s[g, pl.ds(start, AR), :]
        acc = acc + jnp.where(even1, pltpu.roll(acc, 127, 1), pltpu.roll(acc, 1, 1))
        acc = acc + jnp.where(even16, pltpu.roll(acc, 112, 1), pltpu.roll(acc, 16, 1))
        acc = acc * (DH ** -0.5)
        if w:
            acc = jnp.where(pos >= DIL * w, acc, -1e9)
        logits.append(acc)
    m = logits[0]
    for w in range(1, WIN):
        m = jnp.maximum(m, logits[w])
    e = [jnp.exp(l - m) for l in logits]
    den = e[0]
    for w in range(1, WIN):
        den = den + e[w]
    inv = 1.0 / den
    p = [x * inv for x in e]
    for g in range(NG):
        acc = p[0] * v_s[g, pl.ds(r + HALO, AR), :]
        for w in range(1, WIN):
            acc = acc + p[w] * v_s[g, pl.ds(r + (HALO - DIL * w), AR), :]
        o_s[pl.ds(r, AR), g * 128:(g + 1) * 128] = acc.astype(BF16)


def _kernel(x_ref, c_ref, wqkv_hbm, wo_hbm, wg_hbm, wu_hbm, wd_hbm, wmod_hbm, out_ref,
            wmod_s, wqkv_s, wo_raw, wo_s, wg_s, wu_s, wd_s, mod_s,
            q_s, k_s, v_s, o_s, x1_s, h2_s, act_s, sems):
    t = pl.program_id(0)

    def mod_copy(i):
        return pltpu.make_async_copy(wmod_hbm.at[:, pl.ds(i * D, D)], wmod_s.at[i], sems.at[i])

    def qkv_copy(i):
        return pltpu.make_async_copy(wqkv_hbm.at[:, pl.ds(i * D, D)], wqkv_s.at[i], sems.at[6 + i])

    def wo_copies():
        return [pltpu.make_async_copy(wo_hbm.at[:, pl.ds(g * 128, 128)], wo_raw.at[g], sems.at[9])
                for g in range(NG)]

    def gate_copy(f):
        return pltpu.make_async_copy(wg_hbm.at[:, pl.ds(f * FC, FC)], wg_s.at[f], sems.at[10 + f])

    def up_copy(f):
        return pltpu.make_async_copy(wu_hbm.at[:, pl.ds(f * FC, FC)], wu_s.at[f], sems.at[10 + NF + f])

    def down_copy(n):
        return pltpu.make_async_copy(wd_hbm.at[:, pl.ds(n * NC, NC)], wd_s.at[n], sems.at[10 + 2 * NF + n])

    def compute_mod(i):
        cc = c_ref[...]
        sc = jnp.broadcast_to(cc * jax.nn.sigmoid(cc), (16, D)).astype(BF16)
        mod_s[i] = jnp.dot(sc, wmod_s[i], preferred_element_type=F32)[0:8]

    first = t == 0

    @pl.when(first)
    def _():
        mod_copy(0).start()
        mod_copy(1).start()
        qkv_copy(0).start()
        k_s[:, 0:HALO, :] = jnp.zeros((NG, HALO, 128), F32)
        v_s[:, 0:HALO, :] = jnp.zeros((NG, HALO, 128), F32)
        mod_copy(0).wait()
        qkv_copy(1).start()
        compute_mod(0)
        mod_copy(1).wait()
        qkv_copy(2).start()
        compute_mod(1)

    @pl.when(jnp.logical_and(t > 0, t < NT))
    def _():
        k_s[:, 0:HALO, :] = k_s[:, TM:TM + HALO, :]
        v_s[:, 0:HALO, :] = v_s[:, TM:TM + HALO, :]

    @pl.when(t < NT)
    def _():
        h = _layernorm(x_ref[...].astype(F32)) * (1.0 + mod_s[1, 0:1, :]) + mod_s[0, 0:1, :]
        o_s[...] = h.astype(BF16)
        for i, (dst, off) in enumerate(((q_s, 0), (k_s, HALO), (v_s, HALO))):
            @pl.when(first)
            def _():
                qkv_copy(i).wait()
                if i == 0:
                    mod_copy(2).start()
                    for cp in wo_copies():
                        cp.start()
                elif i == 1:
                    mod_copy(3).start()
                    mod_copy(4).start()
                else:
                    for f in range(2):
                        gate_copy(f).start()
                        up_copy(f).start()
                _permute_columns(wqkv_s.at[i])

            y = jnp.dot(o_s[...], wqkv_s[i], preferred_element_type=F32)
            for g in range(NG):
                dst[g, off:off + TM, :] = y[:, g * 128:(g + 1) * 128]

    @pl.when(first)
    def _():
        for f in range(2, NF):
            gate_copy(f).start()
            up_copy(f).start()

        def body(i, carry):
            _attention_block(pl.multiple_of(i * AR, AR), 0, q_s, k_s, v_s, o_s)
            return carry

        lax.fori_loop(0, TM // AR, body, 0)
        mod_copy(5).start()
        for n in range(D // NC):
            down_copy(n).start()
        mod_copy(2).wait()
        compute_mod(2)
        for cp in wo_copies():
            cp.wait()
        _permute_rows(wo_raw, wo_s)
        mod_copy(3).wait()
        compute_mod(3)
        mod_copy(4).wait()
        compute_mod(4)

    @pl.when(t > 0)
    def _():
        def ffn_body(f, carry):
            @pl.when(t == 1)
            def _():
                gate_copy(f).wait()
                up_copy(f).wait()

            h2 = h2_s[...]
            g = jnp.dot(h2, wg_s[f], preferred_element_type=F32)
            u = jnp.dot(h2, wu_s[f], preferred_element_type=F32)
            act_s[f] = (g * jax.nn.sigmoid(g) * u).astype(BF16)
            for a in range(ATT_PER_F):
                blk = jnp.minimum(f * ATT_PER_F + a, TM // AR - 1)
                _attention_block(pl.multiple_of(blk * AR, AR), t * TM, q_s, k_s, v_s, o_s)
            return carry

        lax.fori_loop(0, NF, ffn_body, 0)

        @pl.when(t == 1)
        def _():
            mod_copy(5).wait()
            compute_mod(5)
            for n in range(D // NC):
                down_copy(n).wait()

        for n in range(D // NC):
            y = jnp.dot(act_s[0], wd_s[n, 0:FC, :], preferred_element_type=F32)
            for f in range(1, NF):
                y = y + jnp.dot(act_s[f], wd_s[n, f * FC:(f + 1) * FC, :], preferred_element_type=F32)
            cs = slice(n * NC, (n + 1) * NC)
            out_ref[:, cs] = (x1_s[:, cs] + mod_s[5, 0:1, cs] * y).astype(out_ref.dtype)

    @pl.when(t < NT)
    def _():
        a = jnp.dot(o_s[...], wo_s[...], preferred_element_type=F32)
        x1 = x_ref[...].astype(F32) + mod_s[2, 0:1, :] * a
        x1_s[...] = x1
        h2_s[...] = (_layernorm(x1) * (1.0 + mod_s[4, 0:1, :]) + mod_s[3, 0:1, :]).astype(BF16)


@jax.jit
def pallas_adaLN_cond__sliding_local_dilated__swiglu_ffn__prompt_kernel(
    A_x: jax.Array,
    A_wqkv: jax.Array,
    A_wo: jax.Array,
    B_x: jax.Array,
    B_w_gate: jax.Array,
    B_w_up: jax.Array,
    B_w_down: jax.Array,
    c: jax.Array,
    w_mod: jax.Array,
):
    del B_x
    hbm = pl.BlockSpec(memory_space=pl.ANY)
    out = pl.pallas_call(
        _kernel,
        grid=(NT + 1,),
        in_specs=[
            pl.BlockSpec((TM, D), lambda t: (jnp.minimum(t, NT - 1), 0)),
            pl.BlockSpec((1, D), lambda t: (0, 0)),
            hbm, hbm, hbm, hbm, hbm, hbm,
        ],
        out_specs=pl.BlockSpec((TM, D), lambda t: (jnp.maximum(t - 1, 0), 0)),
        out_shape=jax.ShapeDtypeStruct((S, D), A_x.dtype),
        scratch_shapes=[
            pltpu.VMEM((6, D, D), BF16),
            pltpu.VMEM((3, D, D), BF16),
            pltpu.VMEM((NG, D, 128), BF16),
            pltpu.VMEM((D, D), BF16),
            pltpu.VMEM((NF, D, FC), BF16),
            pltpu.VMEM((NF, D, FC), BF16),
            pltpu.VMEM((D // NC, F, NC), BF16),
            pltpu.VMEM((6, 8, D), F32),
            pltpu.VMEM((NG, TM, 128), F32),
            pltpu.VMEM((NG, HALO + TM, 128), F32),
            pltpu.VMEM((NG, HALO + TM, 128), F32),
            pltpu.VMEM((TM, D), BF16),
            pltpu.VMEM((TM, D), F32),
            pltpu.VMEM((TM, D), BF16),
            pltpu.VMEM((NF, TM, FC), BF16),
            pltpu.SemaphoreType.DMA((10 + 2 * NF + D // NC,)),
        ],
        compiler_params=pltpu.CompilerParams(
            dimension_semantics=("arbitrary",),
            vmem_limit_bytes=100 * 1024 * 1024,
        ),
    )(A_x.reshape(S, D), c.astype(F32), A_wqkv, A_wo, B_w_gate, B_w_up, B_w_down, w_mod)
    return out.reshape(A_x.shape)
```

```python
import jax
import jax.numpy as jnp
from jax import lax
from jax.experimental import pallas as pl
from jax.experimental.pallas import tpu as pltpu

S, D, F = 2048, 1024, 3584
H, DH, WIN, DIL = 32, 32, 8, 2
TM = 512
NT = S // TM
FC = 512
NF = F // FC
NC = 256
HALO = 16
AR = 16
NG = D // 128
ATT_PER_F = -(-(TM // AR) // NF)
EPS = 1e-5
F32, BF16 = jnp.float32, jnp.bfloat16


def _layernorm(x):
    m = jnp.mean(x, axis=-1, keepdims=True)
    xc = x - m
    v = jnp.mean(xc * xc, axis=-1, keepdims=True)
    return xc * lax.rsqrt(v + EPS)


def _permute_columns(w_ref):
    w32 = w_ref.bitcast(jnp.uint32)
    rows = 32
    field = lax.broadcasted_iota(jnp.int32, (rows, 128), 1) >> 1

    def body(i, carry):
        r = pl.multiple_of(i * rows, rows)
        cols = [w32[pl.ds(r, rows), g * 128:(g + 1) * 128] for g in range(NG)]
        cols = [pltpu.roll(x, 2 * g, 1) if g else x for g, x in enumerate(cols)]
        cols = [cols[-g % NG] for g in range(NG)]
        for b in (1, 2, 4):
            bit = (field & b) != 0
            cols = [jnp.where(bit, cols[(g - b) % NG], cols[g]) for g in range(NG)]
        for g in range(NG):
            w32[pl.ds(r, rows), g * 128:(g + 1) * 128] = (
                pltpu.roll(cols[g], 128 - 2 * g, 1) if g else cols[g])
        return carry

    lax.fori_loop(0, D // 2 // rows, body, 0)


def _permute_rows(src_ref, dst_ref):
    s32 = src_ref.bitcast(jnp.uint32)
    d32 = dst_ref.bitcast(jnp.uint32)
    for g in range(NG):
        for j in range(8):
            for m in range(8):
                d32[j * 64 + m * 8:j * 64 + m * 8 + 8, g * 128:(g + 1) * 128] = (
                    s32[g, pl.ds(m * 8 + j, 8, stride=64), :])


def _attention_block(r, pos0, qkv_s, o_s):
    lane = lax.broadcasted_iota(jnp.int32, (AR, 128), 1)
    pos = lax.broadcasted_iota(jnp.int32, (AR, 128), 0) + (pos0 + r)
    even1 = (lane & 1) == 0
    even16 = (lane & 16) == 0
    q = [qkv_s[0, g, pl.ds(r + HALO, AR), :] for g in range(NG)]
    logits = []
    for w in range(WIN):
        start = r + (HALO - DIL * w)
        acc = q[0] * qkv_s[1, 0, pl.ds(start, AR), :]
        for g in range(1, NG):
            acc = acc + q[g] * qkv_s[1, g, pl.ds(start, AR), :]
        acc = acc + jnp.where(even1, pltpu.roll(acc, 127, 1), pltpu.roll(acc, 1, 1))
        acc = acc + jnp.where(even16, pltpu.roll(acc, 112, 1), pltpu.roll(acc, 16, 1))
        acc = acc * (DH ** -0.5)
        if w:
            acc = jnp.where(pos >= DIL * w, acc, -1e9)
        logits.append(acc)
    m = logits[0]
    for w in range(1, WIN):
        m = jnp.maximum(m, logits[w])
    e = [jnp.exp(l - m) for l in logits]
    den = e[0]
    for w in range(1, WIN):
        den = den + e[w]
    inv = 1.0 / den
    p = [x * inv for x in e]
    for g in range(NG):
        acc = p[0] * qkv_s[2, g, pl.ds(r + HALO, AR), :]
        for w in range(1, WIN):
            acc = acc + p[w] * qkv_s[2, g, pl.ds(r + (HALO - DIL * w), AR), :]
        o_s[pl.ds(r, AR), g * 128:(g + 1) * 128] = acc.astype(BF16)


def _kernel(x_ref, xn_ref, c_ref, wqkv_hbm, wo_hbm, wg_hbm, wu_hbm, wd_hbm, wmod_hbm, out_ref,
            wmod_s, wqkv_s, wo_raw, wo_s, wg_s, wu_s, wd_s, mod_s,
            qkv_s, h_s, o_s, x1_s, h2_s, act_s, sems):
    t = pl.program_id(0)
    first = t == 0

    def mod_copy(i):
        return pltpu.make_async_copy(wmod_hbm.at[:, pl.ds(i * D, D)], wmod_s.at[i], sems.at[i])

    def qkv_copy(i):
        return pltpu.make_async_copy(wqkv_hbm.at[:, pl.ds(i * D, D)], wqkv_s.at[i], sems.at[6 + i])

    def wo_copies():
        return [pltpu.make_async_copy(wo_hbm.at[:, pl.ds(g * 128, 128)], wo_raw.at[g], sems.at[9])
                for g in range(NG)]

    def gate_copy(f):
        return pltpu.make_async_copy(wg_hbm.at[:, pl.ds(f * FC, FC)], wg_s.at[f], sems.at[10 + f])

    def up_copy(f):
        return pltpu.make_async_copy(wu_hbm.at[:, pl.ds(f * FC, FC)], wu_s.at[f], sems.at[10 + NF + f])

    def down_copy(n):
        return pltpu.make_async_copy(wd_hbm.at[:, pl.ds(n * NC, NC)], wd_s.at[n], sems.at[10 + 2 * NF + n])

    def compute_mod(lo, hi):
        cc = c_ref[...].astype(F32)
        sc = jnp.broadcast_to(cc * jax.nn.sigmoid(cc), (16, D)).astype(BF16)

        def body(i, carry):
            mod_copy(i).wait()
            mod_s[i] = jnp.dot(sc, wmod_s[i], preferred_element_type=F32)[0:8]
            return carry

        lax.fori_loop(lo, hi, body, 0)

    def modulated_ln(x, shift, scale):
        return (_layernorm(x) * (1.0 + mod_s[scale, 0:1, :]) + mod_s[shift, 0:1, :]).astype(BF16)

    def row_loop(rows, fn):
        def body(i, carry):
            fn(pl.ds(pl.multiple_of(i * rows, rows), rows))
            return carry

        lax.fori_loop(0, TM // rows, body, 0)

    @pl.when(first)
    def _():
        qkv_copy(0).start()
        qkv_copy(1).start()
        qkv_s[1:3, :, 0:HALO, :] = jnp.zeros((2, NG, HALO, 128), F32)

        def body(i, carry):
            qkv_copy(i).wait()

            @pl.when(i == 0)
            def _():
                mod_copy(0).start()
                mod_copy(1).start()

            @pl.when(i == 1)
            def _():
                qkv_copy(2).start()
                mod_copy(2).start()
                for cp in wo_copies():
                    cp.start()

            @pl.when(i == 2)
            def _():
                for j in range(3, 6):
                    mod_copy(j).start()
                for f in range(NF):
                    gate_copy(f).start()
                    up_copy(f).start()

            _permute_columns(wqkv_s.at[i])
            return carry

        lax.fori_loop(0, 3, body, 0)
        compute_mod(0, 2)

        def ln1(rs):
            h_s[rs, :] = modulated_ln(x_ref[rs, :].astype(F32), 0, 1)

        row_loop(64, ln1)

    @pl.when(jnp.logical_and(t > 0, t < NT))
    def _():
        qkv_s[1:3, :, 0:HALO, :] = qkv_s[1:3, :, TM:TM + HALO, :]

    @pl.when(t < NT)
    def _():
        def body(i, carry):
            y = jnp.dot(h_s[...], wqkv_s[i], preferred_element_type=F32)
            for g in range(NG):
                qkv_s[i, g, HALO:HALO + TM, :] = y[:, g * 128:(g + 1) * 128]
            return carry

        lax.fori_loop(0, 3, body, 0)

    @pl.when(first)
    def _():
        for n in range(D // NC):
            down_copy(n).start()

        def body(i, carry):
            _attention_block(pl.multiple_of(i * AR, AR), 0, qkv_s, o_s)
            return carry

        lax.fori_loop(0, TM // AR, body, 0)
        compute_mod(2, 6)
        for cp in wo_copies():
            cp.wait()
        _permute_rows(wo_raw, wo_s)

    @pl.when(t > 0)
    def _():
        def body(f, carry):
            @pl.when(t == 1)
            def _():
                gate_copy(f).wait()
                up_copy(f).wait()

            h2 = h2_s[...]
            g = jnp.dot(h2, wg_s[f], preferred_element_type=F32)
            u = jnp.dot(h2, wu_s[f], preferred_element_type=F32)
            act_s[f] = (g * jax.nn.sigmoid(g) * u).astype(BF16)
            for a in range(ATT_PER_F):
                blk = jnp.minimum(f * ATT_PER_F + a, TM // AR - 1)
                _attention_block(pl.multiple_of(blk * AR, AR), t * TM, qkv_s, o_s)
            return carry

        lax.fori_loop(0, NF, body, 0)

    slot = t % 2

    @pl.when(t < NT)
    def _():
        def proj(rs):
            a = jnp.dot(o_s[rs, :], wo_s[...], preferred_element_type=F32)
            x1_s[slot, rs, :] = x_ref[rs, :].astype(F32) + mod_s[2, 0:1, :] * a

        row_loop(256, proj)

    def next_norms(rs, cur):
        h2_s[rs, :] = modulated_ln(x1_s[cur, rs, :], 3, 4)
        h_s[rs, :] = modulated_ln(xn_ref[rs, :].astype(F32), 0, 1)

    @pl.when(first)
    def _():
        row_loop(64, lambda rs: next_norms(rs, 0))
        for n in range(D // NC):
            down_copy(n).wait()

    @pl.when(t > 0)
    def _():
        cur = jnp.minimum(t, NT - 1) % 2

        def body(n, carry):
            y = jnp.dot(act_s[0], wd_s[n, 0:FC, :], preferred_element_type=F32)
            for f in range(1, NF):
                y = y + jnp.dot(act_s[f], wd_s[n, f * FC:(f + 1) * FC, :], preferred_element_type=F32)
            cs = pl.ds(pl.multiple_of(n * NC, NC), NC)
            out_ref[:, cs] = (x1_s[1 - slot, :, cs] + mod_s[5, 0:1, cs] * y).astype(out_ref.dtype)
            rows = TM // (D // NC)
            next_norms(pl.ds(pl.multiple_of(n * rows, rows), rows), cur)
            return carry

        lax.fori_loop(0, D // NC, body, 0)


@jax.jit
def pallas_adaLN_cond__sliding_local_dilated__swiglu_ffn__prompt_kernel(
    A_x: jax.Array,
    A_wqkv: jax.Array,
    A_wo: jax.Array,
    B_x: jax.Array,
    B_w_gate: jax.Array,
    B_w_up: jax.Array,
    B_w_down: jax.Array,
    c: jax.Array,
    w_mod: jax.Array,
):
    del B_x
    x = A_x.reshape(S, D)
    hbm = pl.BlockSpec(memory_space=pl.ANY)
    out = pl.pallas_call(
        _kernel,
        grid=(NT + 1,),
        in_specs=[
            pl.BlockSpec((TM, D), lambda t: (jnp.minimum(t, NT - 1), 0)),
            pl.BlockSpec((TM, D), lambda t: (jnp.minimum(t + 1, NT - 1), 0)),
            pl.BlockSpec((1, D), lambda t: (0, 0)),
            hbm, hbm, hbm, hbm, hbm, hbm,
        ],
        out_specs=pl.BlockSpec((TM, D), lambda t: (jnp.maximum(t - 1, 0), 0)),
        out_shape=jax.ShapeDtypeStruct((S, D), A_x.dtype),
        scratch_shapes=[
            pltpu.VMEM((6, D, D), BF16),
            pltpu.VMEM((3, D, D), BF16),
            pltpu.VMEM((NG, D, 128), BF16),
            pltpu.VMEM((D, D), BF16),
            pltpu.VMEM((NF, D, FC), BF16),
            pltpu.VMEM((NF, D, FC), BF16),
            pltpu.VMEM((D // NC, F, NC), BF16),
            pltpu.VMEM((6, 8, D), F32),
            pltpu.VMEM((3, NG, HALO + TM, 128), F32),
            pltpu.VMEM((TM, D), BF16),
            pltpu.VMEM((TM, D), BF16),
            pltpu.VMEM((2, TM, D), F32),
            pltpu.VMEM((TM, D), BF16),
            pltpu.VMEM((NF, TM, FC), BF16),
            pltpu.SemaphoreType.DMA((10 + 2 * NF + D // NC,)),
        ],
        compiler_params=pltpu.CompilerParams(
            dimension_semantics=("arbitrary",),
            vmem_limit_bytes=100 * 1024 * 1024,
        ),
    )(x, x, c, A_wqkv, A_wo, B_w_gate, B_w_up, B_w_down, w_mod)
    return out.reshape(A_x.shape)
```

```python
import jax
import jax.numpy as jnp
from jax import lax
from jax.experimental import pallas as pl
from jax.experimental.pallas import tpu as pltpu

S, D, F = 2048, 1024, 3584
H, DH, WIN, DIL = 32, 32, 8, 2
TM = 512
NT = S // TM
FC = 512
NF = F // FC
NC = 256
HALO = 16
AR = 16
PR = 256
ATT = (2, 2, 2, 2, 0, 0, 0)
NG = D // 128
EPS = 1e-5
LOG2E = 1.4426950408889634
F32, BF16 = jnp.float32, jnp.bfloat16


def _layernorm(x):
    m = jnp.mean(x, axis=-1, keepdims=True)
    xc = x - m
    v = jnp.mean(xc * xc, axis=-1, keepdims=True)
    return xc * lax.rsqrt(v + EPS)


def _permute_columns(w_ref):
    w32 = w_ref.bitcast(jnp.uint32)
    rows = 32
    field = lax.broadcasted_iota(jnp.int32, (rows, 128), 1) >> 1

    def body(i, carry):
        r = pl.multiple_of(i * rows, rows)
        cols = [w32[pl.ds(r, rows), g * 128:(g + 1) * 128] for g in range(NG)]
        cols = [pltpu.roll(x, 2 * g, 1) if g else x for g, x in enumerate(cols)]
        cols = [cols[-g % NG] for g in range(NG)]
        for b in (1, 2, 4):
            bit = (field & b) != 0
            cols = [jnp.where(bit, cols[(g - b) % NG], cols[g]) for g in range(NG)]
        for g in range(NG):
            w32[pl.ds(r, rows), g * 128:(g + 1) * 128] = (
                pltpu.roll(cols[g], 128 - 2 * g, 1) if g else cols[g])
        return carry

    lax.fori_loop(0, D // 2 // rows, body, 0)


def _permute_rows(src_ref, dst_ref):
    s32 = src_ref.bitcast(jnp.uint32)
    d32 = dst_ref.bitcast(jnp.uint32)
    for g in range(NG):
        for j in range(8):
            for m in range(8):
                d32[j * 64 + m * 8:j * 64 + m * 8 + 8, g * 128:(g + 1) * 128] = (
                    s32[g, pl.ds(m * 8 + j, 8, stride=64), :])


def _attention_rows(r0, nblk, qkv_s, o_s, first_tile):
    scale = DH ** -0.5
    partial = []
    for b in range(nblk):
        r = r0 + b * AR
        q = [qkv_s[0, g, pl.ds(r + HALO, AR), :] for g in range(NG)]
        for w in range(WIN):
            start = r + (HALO - DIL * w)
            acc = q[0] * qkv_s[1, 0, pl.ds(start, AR), :]
            for g in range(1, NG):
                acc = acc + q[g] * qkv_s[1, g, pl.ds(start, AR), :]
            partial.append(acc.astype(BF16))
    row = lax.broadcasted_iota(jnp.int32, (128, 128), 0)
    col = lax.broadcasted_iota(jnp.int32, (128, 128), 1)
    same_head = ((row & ~17) == (col & ~17)).astype(F32).astype(BF16)
    full = jnp.dot(jnp.concatenate(partial, axis=0), same_head, preferred_element_type=F32)
    for b in range(nblk):
        r = r0 + b * AR
        logits = []
        for w in range(WIN):
            l = full[(b * WIN + w) * AR:(b * WIN + w + 1) * AR]
            if w and first_tile:
                pos = lax.broadcasted_iota(jnp.int32, (AR, 128), 0) + r
                l = jnp.where(pos >= DIL * w, l, -1e9 / scale)
            logits.append(l)
        m = logits[0]
        for w in range(1, WIN):
            m = jnp.maximum(m, logits[w])
        e = [jnp.exp2((l - m) * (scale * LOG2E)) for l in logits]
        den = e[0]
        for w in range(1, WIN):
            den = den + e[w]
        inv = 1.0 / den
        p = [x * inv for x in e]
        for g in range(NG):
            acc = p[0] * qkv_s[2, g, pl.ds(r + HALO, AR), :]
            for w in range(1, WIN):
                acc = acc + p[w] * qkv_s[2, g, pl.ds(r + (HALO - DIL * w), AR), :]
            o_s[pl.ds(r, AR), g * 128:(g + 1) * 128] = acc.astype(BF16)


def _kernel(x_ref, xn_ref, c_ref, wqkv_hbm, wo_hbm, wg_hbm, wu_hbm, wd_hbm, wmod_hbm, out_ref,
            wmod_s, wqkv_s, wo_raw, wo_s, wg_s, wu_s, wd_s, mod_s,
            qkv_s, h_s, o_s, x1_s, h2_s, act_s, sems):
    t = pl.program_id(0)
    first = t == 0

    def mod_copy(i):
        return pltpu.make_async_copy(wmod_hbm.at[:, pl.ds(i * D, D)], wmod_s.at[i], sems.at[i])

    def qkv_copy(i):
        return pltpu.make_async_copy(wqkv_hbm.at[:, pl.ds(i * D, D)], wqkv_s.at[i], sems.at[6 + i])

    def wo_copies():
        return [pltpu.make_async_copy(wo_hbm.at[:, pl.ds(g * 128, 128)], wo_raw.at[g], sems.at[9])
                for g in range(NG)]

    def gate_copy(f):
        return pltpu.make_async_copy(wg_hbm.at[:, pl.ds(f * FC, FC)], wg_s.at[f], sems.at[10 + f])

    def up_copy(f):
        return pltpu.make_async_copy(wu_hbm.at[:, pl.ds(f * FC, FC)], wu_s.at[f], sems.at[10 + NF + f])

    def down_copy(n):
        return pltpu.make_async_copy(wd_hbm.at[:, pl.ds(n * NC, NC)], wd_s.at[n], sems.at[10 + 2 * NF + n])

    def compute_mod(lo, hi):
        cc = c_ref[...].astype(F32)
        sc = jnp.broadcast_to(cc * jax.nn.sigmoid(cc), (16, D)).astype(BF16)

        def body(i, carry):
            mod_copy(i).wait()
            mod_s[i] = jnp.dot(sc, wmod_s[i], preferred_element_type=F32)[0:8]
            return carry

        lax.fori_loop(lo, hi, body, 0)

    def modulated_ln(x, shift, scale):
        return (_layernorm(x) * (1.0 + mod_s[scale, 0:1, :]) + mod_s[shift, 0:1, :]).astype(BF16)

    def norm1(ref, slot, rs):
        h_s[slot, rs, :] = modulated_ln(ref[rs, :].astype(F32), 0, 1)

    def norm2(rs):
        h2_s[rs, :] = modulated_ln(x1_s[rs, :], 3, 4)

    def row_loop(rows, fn):
        def body(i, carry):
            fn(pl.ds(pl.multiple_of(i * rows, rows), rows))
            return carry

        lax.fori_loop(0, TM // rows, body, 0)

    @pl.when(first)
    def _():
        qkv_copy(0).start()
        qkv_copy(1).start()
        qkv_s[1:3, :, 0:HALO, :] = jnp.zeros((2, NG, HALO, 128), F32)

        def body(i, carry):
            qkv_copy(i).wait()

            @pl.when(i == 0)
            def _():
                mod_copy(0).start()
                mod_copy(1).start()

            @pl.when(i == 1)
            def _():
                qkv_copy(2).start()
                mod_copy(2).start()
                for cp in wo_copies():
                    cp.start()

            @pl.when(i == 2)
            def _():
                for j in range(3, 6):
                    mod_copy(j).start()
                for f in range(NF):
                    gate_copy(f).start()
                    up_copy(f).start()

            _permute_columns(wqkv_s.at[i])
            return carry

        lax.fori_loop(0, 3, body, 0)
        compute_mod(0, 2)

        row_loop(64, lambda rs: norm1(x_ref, 0, rs))

    @pl.when(jnp.logical_and(t > 0, t < NT))
    def _():
        qkv_s[1:3, :, 0:HALO, :] = qkv_s[1:3, :, TM:TM + HALO, :]

    @pl.when(t < NT)
    def _():
        def body(i, carry):
            rows = -(-TM // (3 * 16)) * 16
            rs = pl.ds(pl.multiple_of(jnp.minimum(i * rows, TM - rows), 16), rows)
            norm2(rs)
            y = jnp.dot(h_s[t % 2], wqkv_s[i], preferred_element_type=F32)
            norm1(xn_ref, (t + 1) % 2, rs)
            for g in range(NG):
                qkv_s[i, g, HALO:HALO + TM, :] = y[:, g * 128:(g + 1) * 128]
            return carry

        lax.fori_loop(0, 3, body, 0)

    @pl.when(t == NT)
    def _():
        row_loop(64, norm2)

    @pl.when(first)
    def _():
        for n in range(D // NC):
            down_copy(n).start()

        def body(i, carry):
            _attention_rows(pl.multiple_of(i * (4 * AR), 4 * AR), 4, qkv_s, o_s, True)
            return carry

        lax.fori_loop(0, TM // (4 * AR), body, 0)
        compute_mod(2, 6)
        for cp in wo_copies():
            cp.wait()
        _permute_rows(wo_raw, wo_s)

    @pl.when(t > 0)
    def _():
        def gate_up(f, carry):
            @pl.when(t == 1)
            def _():
                gate_copy(f).wait()
                up_copy(f).wait()

            h2 = h2_s[...]
            g = jnp.dot(h2, wg_s[f], preferred_element_type=F32)
            u = jnp.dot(h2, wu_s[f], preferred_element_type=F32)
            act_s[f] = (g * jax.nn.sigmoid(g) * u).astype(BF16)
            return carry

        lax.fori_loop(0, NF, gate_up, 0)

        def down(n, carry):
            @pl.when(t == 1)
            def _():
                down_copy(n).wait()

            r = n * (TM // (D // NC))
            y = None
            for f in range(NF):
                part = jnp.dot(act_s[f], wd_s[n, f * FC:(f + 1) * FC, :], preferred_element_type=F32)
                y = part if f == 0 else y + part
                if ATT[f]:
                    _attention_rows(pl.multiple_of(r, AR), ATT[f], qkv_s, o_s, False)
                    r = r + ATT[f] * AR
            cs = pl.ds(pl.multiple_of(n * NC, NC), NC)
            out_ref[:, cs] = (x1_s[:, cs] + mod_s[5, 0:1, cs] * y).astype(out_ref.dtype)
            return carry

        lax.fori_loop(0, D // NC, down, 0)

    @pl.when(t < NT)
    def _():
        def proj(rs):
            a = jnp.dot(o_s[rs, :], wo_s[...], preferred_element_type=F32)
            x1_s[rs, :] = x_ref[rs, :].astype(F32) + mod_s[2, 0:1, :] * a

        row_loop(PR, proj)


@jax.jit
def pallas_adaLN_cond__sliding_local_dilated__swiglu_ffn__prompt_kernel(
    A_x: jax.Array,
    A_wqkv: jax.Array,
    A_wo: jax.Array,
    B_x: jax.Array,
    B_w_gate: jax.Array,
    B_w_up: jax.Array,
    B_w_down: jax.Array,
    c: jax.Array,
    w_mod: jax.Array,
):
    del B_x
    x = A_x.reshape(S, D)
    hbm = pl.BlockSpec(memory_space=pl.ANY)
    out = pl.pallas_call(
        _kernel,
        grid=(NT + 1,),
        in_specs=[
            pl.BlockSpec((TM, D), lambda t: (jnp.minimum(t, NT - 1), 0)),
            pl.BlockSpec((TM, D), lambda t: (jnp.minimum(t + 1, NT - 1), 0)),
            pl.BlockSpec((1, D), lambda t: (0, 0)),
            hbm, hbm, hbm, hbm, hbm, hbm,
        ],
        out_specs=pl.BlockSpec((TM, D), lambda t: (jnp.maximum(t - 1, 0), 0)),
        out_shape=jax.ShapeDtypeStruct((S, D), A_x.dtype),
        scratch_shapes=[
            pltpu.VMEM((6, D, D), BF16),
            pltpu.VMEM((3, D, D), BF16),
            pltpu.VMEM((NG, D, 128), BF16),
            pltpu.VMEM((D, D), BF16),
            pltpu.VMEM((NF, D, FC), BF16),
            pltpu.VMEM((NF, D, FC), BF16),
            pltpu.VMEM((D // NC, F, NC), BF16),
            pltpu.VMEM((6, 8, D), F32),
            pltpu.VMEM((3, NG, HALO + TM, 128), F32),
            pltpu.VMEM((2, TM, D), BF16),
            pltpu.VMEM((TM, D), BF16),
            pltpu.VMEM((TM, D), F32),
            pltpu.VMEM((TM, D), BF16),
            pltpu.VMEM((NF, TM, FC), BF16),
            pltpu.SemaphoreType.DMA((10 + 2 * NF + D // NC,)),
        ],
        compiler_params=pltpu.CompilerParams(
            dimension_semantics=("arbitrary",),
            vmem_limit_bytes=100 * 1024 * 1024,
        ),
    )(x, x, c, A_wqkv, A_wo, B_w_gate, B_w_up, B_w_down, w_mod)
    return out.reshape(A_x.shape)
```

```python
import jax
import jax.numpy as jnp
from jax import lax
from jax.experimental import pallas as pl
from jax.experimental.pallas import tpu as pltpu

S, D, F = 2048, 1024, 3584
H, DH, WIN, DIL = 32, 32, 8, 2
TM = 512
NT = S // TM
FC = 512
NF = F // FC
NC = 256
HALO = 16
AR = 16
PR = 256
ATT = (2, 2, 2, 2, 0, 0, 0)
QP = 4
AHEAD = 4
NG = D // 128
EPS = 1e-5
LOG2E = 1.4426950408889634
F32, BF16 = jnp.float32, jnp.bfloat16


def _layernorm(x):
    m = jnp.mean(x, axis=-1, keepdims=True)
    xc = x - m
    v = jnp.mean(xc * xc, axis=-1, keepdims=True)
    return xc * lax.rsqrt(v + EPS)


def _permute_columns(w_ref, rs):
    shift = (lax.broadcasted_iota(jnp.int32, (128, 128), 1)
             - lax.broadcasted_iota(jnp.int32, (128, 128), 0)) & 127

    def roll(x, n):
        if n == 0:
            return x
        rot = (shift == n % 128).astype(F32).astype(BF16)
        return jnp.dot(x, rot, preferred_element_type=F32).astype(BF16)

    cols = [roll(w_ref[rs, g * 128:(g + 1) * 128], 2 * g) for g in range(NG)]
    cols = [pltpu.bitcast(cols[-g % NG], jnp.uint32) for g in range(NG)]
    field = lax.broadcasted_iota(jnp.int32, cols[0].shape, 1) >> 1
    for b in (1, 2, 4):
        bit = (field & b) != 0
        cols = [jnp.where(bit, cols[(g - b) % NG], cols[g]) for g in range(NG)]
    for g in range(NG):
        w_ref[rs, g * 128:(g + 1) * 128] = roll(pltpu.bitcast(cols[g], BF16), -2 * g)


def _permute_rows(src_ref, dst_ref, g):
    s32 = src_ref.bitcast(jnp.uint32)
    d32 = dst_ref.bitcast(jnp.uint32)
    cs = pl.ds(pl.multiple_of(g * 128, 128), 128)
    for j in range(8):
        for m in range(8):
            d32[j * 64 + m * 8:j * 64 + m * 8 + 8, cs] = s32[g, pl.ds(m * 8 + j, 8, stride=64), :]


def _attention_rows(r0, nblk, qkv_s, o_s, first_tile):
    scale = DH ** -0.5
    partial = []
    for b in range(nblk):
        r = r0 + b * AR
        q = [qkv_s[0, g, pl.ds(r + HALO, AR), :] for g in range(NG)]
        for w in range(WIN):
            start = r + (HALO - DIL * w)
            acc = q[0] * qkv_s[1, 0, pl.ds(start, AR), :]
            for g in range(1, NG):
                acc = acc + q[g] * qkv_s[1, g, pl.ds(start, AR), :]
            partial.append(acc.astype(BF16))
    row = lax.broadcasted_iota(jnp.int32, (128, 128), 0)
    col = lax.broadcasted_iota(jnp.int32, (128, 128), 1)
    same_head = ((row & ~17) == (col & ~17)).astype(F32).astype(BF16)
    full = jnp.dot(jnp.concatenate(partial, axis=0), same_head, preferred_element_type=F32)
    for b in range(nblk):
        r = r0 + b * AR
        logits = []
        for w in range(WIN):
            l = full[(b * WIN + w) * AR:(b * WIN + w + 1) * AR]
            if w and first_tile:
                pos = lax.broadcasted_iota(jnp.int32, (AR, 128), 0) + r
                l = jnp.where(pos >= DIL * w, l, -1e9 / scale)
            logits.append(l)
        m = logits[0]
        for w in range(1, WIN):
            m = jnp.maximum(m, logits[w])
        e = [jnp.exp2((l - m) * (scale * LOG2E)) for l in logits]
        den = e[0]
        for w in range(1, WIN):
            den = den + e[w]
        inv = 1.0 / den
        p = [x * inv for x in e]
        for g in range(NG):
            acc = p[0] * qkv_s[2, g, pl.ds(r + HALO, AR), :]
            for w in range(1, WIN):
                acc = acc + p[w] * qkv_s[2, g, pl.ds(r + (HALO - DIL * w), AR), :]
            o_s[pl.ds(r, AR), g * 128:(g + 1) * 128] = acc.astype(BF16)


def _kernel(x_hbm, c_hbm, wqkv_hbm, wo_hbm, wg_hbm, wu_hbm, wd_hbm, wmod_hbm, out_ref,
            x_s, c_s, wmod_s, wqkv_s, wo_raw, wo_s, wg_s, wu_s, wd_s, mod_s,
            qkv_s, h_s, o_s, x1_s, h2_s, act_s, sems, qsems, xsems):
    t = pl.program_id(0)
    first = t == 0

    def mod_copy(i):
        return pltpu.make_async_copy(wmod_hbm.at[:, pl.ds(pl.multiple_of(i * D, D), D)], wmod_s.at[i], sems.at[i])

    def qkv_copy(p):
        rs = pl.ds(pl.multiple_of((p % QP) * (D // QP), D // QP), D // QP)
        return pltpu.make_async_copy(wqkv_hbm.at[rs, pl.ds(pl.multiple_of((p // QP) * D, D), D)],
                                     wqkv_s.at[p // QP, rs], qsems.at[p])

    def x_copy(i):
        return pltpu.make_async_copy(x_hbm.at[pl.ds(pl.multiple_of(i * TM, TM), TM)], x_s.at[i], xsems.at[i])

    def c_copy():
        return pltpu.make_async_copy(c_hbm, c_s, sems.at[6])

    def wo_copies():
        return [pltpu.make_async_copy(wo_hbm.at[:, pl.ds(g * 128, 128)], wo_raw.at[g], sems.at[9])
                for g in range(NG)]

    def gate_copy(f):
        return pltpu.make_async_copy(wg_hbm.at[:, pl.ds(pl.multiple_of(f * FC, FC), FC)], wg_s.at[f], sems.at[10 + f])

    def up_copy(f):
        return pltpu.make_async_copy(wu_hbm.at[:, pl.ds(pl.multiple_of(f * FC, FC), FC)], wu_s.at[f], sems.at[10 + NF + f])

    def down_copy(n):
        return pltpu.make_async_copy(wd_hbm.at[:, pl.ds(n * NC, NC)], wd_s.at[n], sems.at[10 + 2 * NF + n])

    def compute_mod(i, cs):
        cc = c_s[...].astype(F32)
        sc = jnp.broadcast_to(cc * jax.nn.sigmoid(cc), (16, D)).astype(BF16)
        mod_s[i, :, cs] = jnp.dot(sc, wmod_s[i, :, cs], preferred_element_type=F32)[0:8]

    def modulated_ln(x, shift, scale):
        return (_layernorm(x) * (1.0 + mod_s[scale, 0:1, :]) + mod_s[shift, 0:1, :]).astype(BF16)

    def norm1(tile, slot, rs):
        h_s[slot, rs, :] = modulated_ln(x_s[tile, rs, :].astype(F32), 0, 1)

    def norm2(rs):
        h2_s[rs, :] = modulated_ln(x1_s[rs, :], 3, 4)

    def row_loop(rows, fn):
        def body(i, carry):
            fn(pl.ds(pl.multiple_of(i * rows, rows), rows))
            return carry

        lax.fori_loop(0, TM // rows, body, 0)

    @pl.when(first)
    def _():
        for p in range(AHEAD):
            qkv_copy(p).start()
        c_copy().start()
        qkv_s[1:3, :, 0:HALO, :] = jnp.zeros((2, NG, HALO, 128), F32)

        def perm_body(p, carry):
            qkv_copy(p).wait()
            left = 3 * QP - 1 - p
            pl.when(left >= AHEAD)(lambda: qkv_copy(p + AHEAD).start())
            pl.when(left == AHEAD + 1)(mod_copy(0).start)
            pl.when(left == AHEAD - 1)(x_copy(0).start)
            pl.when(left == AHEAD - 2)(mod_copy(1).start)
            rows = D // QP
            _permute_columns(wqkv_s.at[p // QP], pl.ds(pl.multiple_of((p % QP) * rows, rows), rows))
            return carry

        lax.fori_loop(0, 3 * QP, perm_body, 0)
        c_copy().wait()

        def mod_body(i, carry):
            mod_copy(i).wait()

            @pl.when(i == 0)
            def _():
                x_copy(1).start()

            @pl.when(i == 1)
            def _():
                for cp in wo_copies():
                    cp.start()
                for j in range(2, 6):
                    mod_copy(j).start()

            compute_mod(i, slice(None))
            return carry

        lax.fori_loop(0, 2, mod_body, 0)
        x_copy(0).wait()
        row_loop(64, lambda rs: norm1(0, 0, rs))

    @pl.when(t + 1 < NT)
    def _():
        x_copy(t + 1).wait()

    @pl.when(jnp.logical_and(t > 0, t < NT))
    def _():
        qkv_s[1:3, :, 0:HALO, :] = qkv_s[1:3, :, TM:TM + HALO, :]

    @pl.when(t < NT)
    def _():
        def body(i, carry):
            @pl.when(jnp.logical_and(first, i > 0))
            def _():
                x_copy(i + 1).start()
                for f in range(2):
                    gate_copy(2 * (i - 1) + f).start()
                    up_copy(2 * (i - 1) + f).start()

            rows = -(-TM // (3 * 16)) * 16
            rs = pl.ds(pl.multiple_of(jnp.minimum(i * rows, TM - rows), 16), rows)
            norm2(rs)
            y = jnp.dot(h_s[t % 2], wqkv_s[i], preferred_element_type=F32)
            norm1(jnp.minimum(t + 1, NT - 1), (t + 1) % 2, rs)
            for g in range(NG):
                qkv_s[i, g, HALO:HALO + TM, :] = y[:, g * 128:(g + 1) * 128]
            return carry

        lax.fori_loop(0, 3, body, 0)

    @pl.when(t == NT)
    def _():
        row_loop(64, norm2)

    @pl.when(first)
    def _():
        for f in range(4, NF):
            gate_copy(f).start()
            up_copy(f).start()
        for n in range(D // NC):
            down_copy(n).start()
        for i in range(2, 6):
            mod_copy(i).wait()
        for cp in wo_copies():
            cp.wait()

        def body(i, carry):
            nblk = TM // AR // NG
            _attention_rows(pl.multiple_of(i * (nblk * AR), nblk * AR), nblk, qkv_s, o_s, True)
            compute_mod(2 + i // 2, pl.ds(pl.multiple_of((i % 2) * (D // 2), D // 2), D // 2))
            _permute_rows(wo_raw, wo_s, i)
            return carry

        lax.fori_loop(0, NG, body, 0)

    @pl.when(t > 0)
    def _():
        def gate_up(f, carry):
            @pl.when(t == 1)
            def _():
                gate_copy(f).wait()
                up_copy(f).wait()

            h2 = h2_s[...]
            g = jnp.dot(h2, wg_s[f], preferred_element_type=F32)
            u = jnp.dot(h2, wu_s[f], preferred_element_type=F32)
            act_s[f] = (g * jax.nn.sigmoid(g) * u).astype(BF16)
            return carry

        lax.fori_loop(0, NF, gate_up, 0)

        def down(n, carry):
            @pl.when(t == 1)
            def _():
                down_copy(n).wait()

            r = n * (TM // (D // NC))
            y = None
            for f in range(NF):
                part = jnp.dot(act_s[f], wd_s[n, f * FC:(f + 1) * FC, :], preferred_element_type=F32)
                y = part if f == 0 else y + part
                if ATT[f]:
                    _attention_rows(pl.multiple_of(r, AR), ATT[f], qkv_s, o_s, False)
                    r = r + ATT[f] * AR
            cs = pl.ds(pl.multiple_of(n * NC, NC), NC)
            out_ref[:, cs] = (x1_s[:, cs] + mod_s[5, 0:1, cs] * y).astype(out_ref.dtype)
            return carry

        lax.fori_loop(0, D // NC, down, 0)

    @pl.when(t < NT)
    def _():
        def proj(rs):
            a = jnp.dot(o_s[rs, :], wo_s[...], preferred_element_type=F32)
            x1_s[rs, :] = x_s[t, rs, :].astype(F32) + mod_s[2, 0:1, :] * a

        row_loop(PR, proj)


@jax.jit
def pallas_adaLN_cond__sliding_local_dilated__swiglu_ffn__prompt_kernel(
    A_x: jax.Array,
    A_wqkv: jax.Array,
    A_wo: jax.Array,
    B_x: jax.Array,
    B_w_gate: jax.Array,
    B_w_up: jax.Array,
    B_w_down: jax.Array,
    c: jax.Array,
    w_mod: jax.Array,
):
    del B_x
    hbm = pl.BlockSpec(memory_space=pl.ANY)
    out = pl.pallas_call(
        _kernel,
        grid=(NT + 1,),
        in_specs=[hbm] * 8,
        out_specs=pl.BlockSpec((TM, D), lambda t: (jnp.maximum(t - 1, 0), 0)),
        out_shape=jax.ShapeDtypeStruct((S, D), A_x.dtype),
        scratch_shapes=[
            pltpu.VMEM((NT, TM, D), BF16),
            pltpu.VMEM((1, D), BF16),
            pltpu.VMEM((6, D, D), BF16),
            pltpu.VMEM((3, D, D), BF16),
            pltpu.VMEM((NG, D, 128), BF16),
            pltpu.VMEM((D, D), BF16),
            pltpu.VMEM((NF, D, FC), BF16),
            pltpu.VMEM((NF, D, FC), BF16),
            pltpu.VMEM((D // NC, F, NC), BF16),
            pltpu.VMEM((6, 8, D), F32),
            pltpu.VMEM((3, NG, HALO + TM, 128), F32),
            pltpu.VMEM((2, TM, D), BF16),
            pltpu.VMEM((TM, D), BF16),
            pltpu.VMEM((TM, D), F32),
            pltpu.VMEM((TM, D), BF16),
            pltpu.VMEM((NF, TM, FC), BF16),
            pltpu.SemaphoreType.DMA((10 + 2 * NF + D // NC,)),
            pltpu.SemaphoreType.DMA((3 * QP,)),
            pltpu.SemaphoreType.DMA((NT,)),
        ],
        compiler_params=pltpu.CompilerParams(
            dimension_semantics=("arbitrary",),
            vmem_limit_bytes=100 * 1024 * 1024,
        ),
    )(A_x.reshape(S, D), c, A_wqkv, A_wo, B_w_gate, B_w_up, B_w_down, w_mod)
    return out.reshape(A_x.shape)
```

```python
import jax
import jax.numpy as jnp
from jax import lax
from jax.experimental import pallas as pl
from jax.experimental.pallas import tpu as pltpu

S, D, F = 2048, 1024, 3584
H, DH, WIN, DIL = 32, 32, 8, 2
TM = 512
NT = S // TM
FC = 512
NF = F // FC
NC = 256
HALO = 16
AR = 16
PR = 256
ATT_G, ATT_D = 5, 0
QP = 4
AHEAD = 4
NG = D // 128
EPS = 1e-5
LOG2E = 1.4426950408889634
F32, BF16 = jnp.float32, jnp.bfloat16


def _layernorm(x):
    m = jnp.mean(x, axis=-1, keepdims=True)
    xc = x - m
    v = jnp.mean(xc * xc, axis=-1, keepdims=True)
    return xc * lax.rsqrt(v + EPS)


def _permute_columns(w_ref, rs):
    shift = (lax.broadcasted_iota(jnp.int32, (128, 128), 1)
             - lax.broadcasted_iota(jnp.int32, (128, 128), 0)) & 127

    def roll(x, n):
        if n == 0:
            return x
        rot = (shift == n % 128).astype(F32).astype(BF16)
        return jnp.dot(x, rot, preferred_element_type=F32).astype(BF16)

    cols = [roll(w_ref[rs, g * 128:(g + 1) * 128], 2 * g) for g in range(NG)]
    cols = [pltpu.bitcast(cols[-g % NG], jnp.uint32) for g in range(NG)]
    field = lax.broadcasted_iota(jnp.int32, cols[0].shape, 1) >> 1
    for b in (1, 2, 4):
        bit = (field & b) != 0
        cols = [jnp.where(bit, cols[(g - b) % NG], cols[g]) for g in range(NG)]
    for g in range(NG):
        w_ref[rs, g * 128:(g + 1) * 128] = roll(pltpu.bitcast(cols[g], BF16), -2 * g)


def _permute_rows(src_ref, dst_ref, g):
    s32 = src_ref.bitcast(jnp.uint32)
    d32 = dst_ref.bitcast(jnp.uint32)
    cs = pl.ds(pl.multiple_of(g * 128, 128), 128)
    for j in range(8):
        for m in range(8):
            d32[j * 64 + m * 8:j * 64 + m * 8 + 8, cs] = s32[g, pl.ds(m * 8 + j, 8, stride=64), :]


def _attention_rows(r0, nblk, qkv_s, o_s, first_tile):
    scale = DH ** -0.5
    partial = []
    for b in range(nblk):
        r = r0 + b * AR
        q = [qkv_s[0, g, pl.ds(r + HALO, AR), :] for g in range(NG)]
        for w in range(WIN):
            start = r + (HALO - DIL * w)
            acc = q[0] * qkv_s[1, 0, pl.ds(start, AR), :]
            for g in range(1, NG):
                acc = acc + q[g] * qkv_s[1, g, pl.ds(start, AR), :]
            partial.append(acc)
    if first_tile:
        row = lax.broadcasted_iota(jnp.int32, (128, 128), 0)
        col = lax.broadcasted_iota(jnp.int32, (128, 128), 1)
        same_head = ((row & ~17) == (col & ~17)).astype(F32).astype(BF16)
        full = jnp.dot(jnp.concatenate(partial, axis=0).astype(BF16), same_head,
                       preferred_element_type=F32)
        full = [full[i * AR:(i + 1) * AR] for i in range(len(partial))]
    else:
        lane = lax.broadcasted_iota(jnp.int32, (AR, 128), 1)
        full = partial
        for sh in (1, 16):
            low = (lane & sh) == 0
            full = [x + jnp.where(low, pltpu.roll(x, 128 - sh, 1), pltpu.roll(x, sh, 1)) for x in full]
    for b in range(nblk):
        r = r0 + b * AR
        logits = []
        for w in range(WIN):
            l = full[b * WIN + w]
            if w and first_tile:
                pos = lax.broadcasted_iota(jnp.int32, (AR, 128), 0) + r
                l = jnp.where(pos >= DIL * w, l, -1e9 / scale)
            logits.append(l)
        m = logits[0]
        for w in range(1, WIN):
            m = jnp.maximum(m, logits[w])
        e = [jnp.exp2((l - m) * (scale * LOG2E)) for l in logits]
        den = e[0]
        for w in range(1, WIN):
            den = den + e[w]
        inv = 1.0 / den
        p = [x * inv for x in e]
        for g in range(NG):
            acc = p[0] * qkv_s[2, g, pl.ds(r + HALO, AR), :]
            for w in range(1, WIN):
                acc = acc + p[w] * qkv_s[2, g, pl.ds(r + (HALO - DIL * w), AR), :]
            o_s[pl.ds(r, AR), g * 128:(g + 1) * 128] = acc.astype(BF16)


def _kernel(x_hbm, c_hbm, wqkv_hbm, wo_hbm, wg_hbm, wu_hbm, wd_hbm, wmod_hbm, out_ref,
            x_s, c_s, wmod_s, wqkv_s, wo_raw, wo_s, wg_s, wu_s, wd_s, mod_s,
            qkv_s, h_s, o_s, x1_s, h2_s, act_s, sems, qsems, xsems):
    t = pl.program_id(0)
    first = t == 0

    def mod_copy(i):
        return pltpu.make_async_copy(wmod_hbm.at[:, pl.ds(pl.multiple_of(i * D, D), D)], wmod_s.at[i], sems.at[i])

    def qkv_copy(p):
        rs = pl.ds(pl.multiple_of((p % QP) * (D // QP), D // QP), D // QP)
        return pltpu.make_async_copy(wqkv_hbm.at[rs, pl.ds(pl.multiple_of((p // QP) * D, D), D)],
                                     wqkv_s.at[p // QP, rs], qsems.at[p])

    def x_copy(i):
        return pltpu.make_async_copy(x_hbm.at[pl.ds(pl.multiple_of(i * TM, TM), TM)], x_s.at[i], xsems.at[i])

    def c_copy():
        return pltpu.make_async_copy(c_hbm, c_s, sems.at[6])

    def wo_copies():
        return [pltpu.make_async_copy(wo_hbm.at[:, pl.ds(g * 128, 128)], wo_raw.at[g], sems.at[9])
                for g in range(NG)]

    def gate_copy(f):
        return pltpu.make_async_copy(wg_hbm.at[:, pl.ds(pl.multiple_of(f * FC, FC), FC)], wg_s.at[f], sems.at[10 + f])

    def up_copy(f):
        return pltpu.make_async_copy(wu_hbm.at[:, pl.ds(pl.multiple_of(f * FC, FC), FC)], wu_s.at[f], sems.at[10 + NF + f])

    def down_copy(n):
        return pltpu.make_async_copy(wd_hbm.at[:, pl.ds(n * NC, NC)], wd_s.at[n], sems.at[10 + 2 * NF + n])

    def compute_mod(i, cs):
        cc = c_s[...].astype(F32)
        sc = jnp.broadcast_to(cc * jax.nn.sigmoid(cc), (16, D)).astype(BF16)
        mod_s[i, :, cs] = jnp.dot(sc, wmod_s[i, :, cs], preferred_element_type=F32)[0:8]

    def modulated_ln(x, shift, scale):
        return (_layernorm(x) * (1.0 + mod_s[scale, 0:1, :]) + mod_s[shift, 0:1, :]).astype(BF16)

    def norm1(tile, slot, rs):
        h_s[slot, rs, :] = modulated_ln(x_s[tile, rs, :].astype(F32), 0, 1)

    def norm2(rs):
        h2_s[rs, :] = modulated_ln(x1_s[rs, :], 3, 4)

    def row_loop(rows, fn):
        def body(i, carry):
            fn(pl.ds(pl.multiple_of(i * rows, rows), rows))
            return carry

        lax.fori_loop(0, TM // rows, body, 0)

    @pl.when(first)
    def _():
        for p in range(AHEAD):
            qkv_copy(p).start()
        c_copy().start()
        qkv_s[1:3, :, 0:HALO, :] = jnp.zeros((2, NG, HALO, 128), F32)

        def perm_body(p, carry):
            qkv_copy(p).wait()
            left = 3 * QP - 1 - p
            pl.when(left >= AHEAD)(lambda: qkv_copy(p + AHEAD).start())
            pl.when(left == AHEAD + 1)(mod_copy(0).start)
            pl.when(left == AHEAD - 1)(x_copy(0).start)
            pl.when(left == AHEAD - 2)(mod_copy(1).start)
            rows = D // QP
            _permute_columns(wqkv_s.at[p // QP], pl.ds(pl.multiple_of((p % QP) * rows, rows), rows))
            return carry

        lax.fori_loop(0, 3 * QP, perm_body, 0)
        c_copy().wait()

        def mod_body(i, carry):
            mod_copy(i).wait()

            @pl.when(i == 0)
            def _():
                x_copy(1).start()

            @pl.when(i == 1)
            def _():
                for cp in wo_copies():
                    cp.start()
                for j in range(2, 6):
                    mod_copy(j).start()

            compute_mod(i, slice(None))
            return carry

        lax.fori_loop(0, 2, mod_body, 0)
        x_copy(0).wait()
        row_loop(64, lambda rs: norm1(0, 0, rs))

    @pl.when(t + 1 < NT)
    def _():
        x_copy(t + 1).wait()

    @pl.when(jnp.logical_and(t > 0, t < NT))
    def _():
        qkv_s[1:3, :, 0:HALO, :] = qkv_s[1:3, :, TM:TM + HALO, :]

    @pl.when(t < NT)
    def _():
        def body(i, carry):
            @pl.when(jnp.logical_and(first, i > 0))
            def _():
                x_copy(i + 1).start()
                for f in range(2):
                    gate_copy(2 * (i - 1) + f).start()
                    up_copy(2 * (i - 1) + f).start()

            rows = -(-TM // (3 * 16)) * 16
            rs = pl.ds(pl.multiple_of(jnp.minimum(i * rows, TM - rows), 16), rows)
            norm2(rs)
            y = jnp.dot(h_s[t % 2], wqkv_s[i], preferred_element_type=F32)
            for g in range(NG):
                qkv_s[i, g, HALO:HALO + TM, :] = y[:, g * 128:(g + 1) * 128]
            return carry

        lax.fori_loop(0, 3, body, 0)

    @pl.when(t == NT)
    def _():
        row_loop(64, norm2)

    @pl.when(first)
    def _():
        for f in range(4, NF):
            gate_copy(f).start()
            up_copy(f).start()
        for n in range(D // NC):
            down_copy(n).start()
        for i in range(2, 6):
            mod_copy(i).wait()
        for cp in wo_copies():
            cp.wait()

        def body(i, carry):
            nblk = TM // AR // NG
            _attention_rows(pl.multiple_of(i * (nblk * AR), nblk * AR), nblk, qkv_s, o_s, True)
            compute_mod(2 + i // 2, pl.ds(pl.multiple_of((i % 2) * (D // 2), D // 2), D // 2))
            _permute_rows(wo_raw, wo_s, i)
            return carry

        lax.fori_loop(0, NG, body, 0)
        row_loop(64, lambda rs: norm1(1, 1, rs))

    @pl.when(t > 0)
    def _():
        def gate_up(f, carry):
            @pl.when(t == 1)
            def _():
                gate_copy(f).wait()
                up_copy(f).wait()

            rows = -(-TM // (NF * 16)) * 16
            norm1(jnp.minimum(t + 1, NT - 1), (t + 1) % 2,
                  pl.ds(pl.multiple_of(jnp.minimum(f * rows, TM - rows), 16), rows))
            for b in range(ATT_G):
                blk = jnp.minimum(f * ATT_G + b, TM // AR - 1)
                _attention_rows(pl.multiple_of(blk * AR, AR), 1, qkv_s, o_s, False)
            g = jnp.dot(h2_s[...], wg_s[f], preferred_element_type=F32)
            u = jnp.dot(h2_s[...], wu_s[f], preferred_element_type=F32)
            act_s[f] = (g * jax.nn.sigmoid(g) * u).astype(BF16)
            return carry

        lax.fori_loop(0, NF, gate_up, 0)

        def down(n, carry):
            @pl.when(t == 1)
            def _():
                down_copy(n).wait()

            for b in range(ATT_D):
                blk = jnp.minimum(NF * ATT_G + n * ATT_D + b, TM // AR - 1)
                _attention_rows(pl.multiple_of(blk * AR, AR), 1, qkv_s, o_s, False)
            y = None
            for f in range(NF):
                part = jnp.dot(act_s[f], wd_s[n, f * FC:(f + 1) * FC, :], preferred_element_type=F32)
                y = part if f == 0 else y + part
            cs = pl.ds(pl.multiple_of(n * NC, NC), NC)
            out_ref[:, cs] = (x1_s[:, cs] + mod_s[5, 0:1, cs] * y).astype(out_ref.dtype)
            return carry

        lax.fori_loop(0, D // NC, down, 0)

    @pl.when(t < NT)
    def _():
        def proj(rs):
            a = jnp.dot(o_s[rs, :], wo_s[...], preferred_element_type=F32)
            x1_s[rs, :] = x_s[t, rs, :].astype(F32) + mod_s[2, 0:1, :] * a

        row_loop(PR, proj)


@jax.jit
def pallas_adaLN_cond__sliding_local_dilated__swiglu_ffn__prompt_kernel(
    A_x: jax.Array,
    A_wqkv: jax.Array,
    A_wo: jax.Array,
    B_x: jax.Array,
    B_w_gate: jax.Array,
    B_w_up: jax.Array,
    B_w_down: jax.Array,
    c: jax.Array,
    w_mod: jax.Array,
):
    del B_x
    hbm = pl.BlockSpec(memory_space=pl.ANY)
    out = pl.pallas_call(
        _kernel,
        grid=(NT + 1,),
        in_specs=[hbm] * 8,
        out_specs=pl.BlockSpec((TM, D), lambda t: (jnp.maximum(t - 1, 0), 0)),
        out_shape=jax.ShapeDtypeStruct((S, D), A_x.dtype),
        scratch_shapes=[
            pltpu.VMEM((NT, TM, D), BF16),
            pltpu.VMEM((1, D), BF16),
            pltpu.VMEM((6, D, D), BF16),
            pltpu.VMEM((3, D, D), BF16),
            pltpu.VMEM((NG, D, 128), BF16),
            pltpu.VMEM((D, D), BF16),
            pltpu.VMEM((NF, D, FC), BF16),
            pltpu.VMEM((NF, D, FC), BF16),
            pltpu.VMEM((D // NC, F, NC), BF16),
            pltpu.VMEM((6, 8, D), F32),
            pltpu.VMEM((3, NG, HALO + TM, 128), F32),
            pltpu.VMEM((2, TM, D), BF16),
            pltpu.VMEM((TM, D), BF16),
            pltpu.VMEM((TM, D), F32),
            pltpu.VMEM((TM, D), BF16),
            pltpu.VMEM((NF, TM, FC), BF16),
            pltpu.SemaphoreType.DMA((10 + 2 * NF + D // NC,)),
            pltpu.SemaphoreType.DMA((3 * QP,)),
            pltpu.SemaphoreType.DMA((NT,)),
        ],
        compiler_params=pltpu.CompilerParams(
            dimension_semantics=("arbitrary",),
            flags={'XLA_TPU_EVENLY_DISTRIBUTE_CRITICAL_NODES': True},
            vmem_limit_bytes=100 * 1024 * 1024,
        ),
    )(A_x.reshape(S, D), c, A_wqkv, A_wo, B_w_gate, B_w_up, B_w_down, w_mod)
    return out.reshape(A_x.shape)
```

```python
import jax
import jax.numpy as jnp
from jax import lax
from jax.experimental import pallas as pl
from jax.experimental.pallas import tpu as pltpu

S, D, F = 2048, 1024, 3584
H, DH, WIN, DIL = 32, 32, 8, 2
TM = 512
NT = S // TM
FC = 512
NF = F // FC
NC = 256
HALO = 16
AR = 16
PR = 512
KP = 8
QP = 4
NG = D // 128
EPS = 1e-5
LOG2E = 1.4426950408889634
F32, BF16 = jnp.float32, jnp.bfloat16


def _layernorm(x):
    m = jnp.mean(x, axis=-1, keepdims=True)
    xc = x - m
    v = jnp.mean(xc * xc, axis=-1, keepdims=True)
    return xc * lax.rsqrt(v + EPS)


def _permute_columns(w_ref, rs, on_mxu):
    shift = (lax.broadcasted_iota(jnp.int32, (128, 128), 1)
             - lax.broadcasted_iota(jnp.int32, (128, 128), 0)) & 127

    def roll(x, n):
        if n == 0:
            return x
        if not on_mxu:
            return pltpu.roll(x, n % 128, 1)
        rot = (shift == n % 128).astype(F32).astype(BF16)
        y = jnp.dot(pltpu.bitcast(x, BF16), rot, preferred_element_type=F32)
        return pltpu.bitcast(y.astype(BF16), jnp.uint32)

    cols = [roll(pltpu.bitcast(w_ref[rs, g * 128:(g + 1) * 128], jnp.uint32), 2 * g) for g in range(NG)]
    cols = [cols[-g % NG] for g in range(NG)]
    field = lax.broadcasted_iota(jnp.int32, cols[0].shape, 1) >> 1
    for b in (1, 2, 4):
        bit = (field & b) != 0
        cols = [jnp.where(bit, cols[(g - b) % NG], cols[g]) for g in range(NG)]
    for g in range(NG):
        w_ref[rs, g * 128:(g + 1) * 128] = pltpu.bitcast(roll(cols[g], -2 * g), BF16)


def _permute_rows(src_ref, dst_ref, g):
    s32 = src_ref.bitcast(jnp.uint32)
    d32 = dst_ref.bitcast(jnp.uint32)
    cs = pl.ds(pl.multiple_of(g * 128, 128), 128)
    for j in range(8):
        for m in range(8):
            d32[j * 64 + m * 8:j * 64 + m * 8 + 8, cs] = s32[g, pl.ds(m * 8 + j, 8, stride=64), :]


def _attention_block(s0, r, qkv_s, o_s, masked):
    scale = DH ** -0.5
    lane = lax.broadcasted_iota(jnp.int32, (AR, 128), 1)

    def window(which, g, w):
        return qkv_s[which, g, pl.ds(s0 + r + (HALO - DIL * w), AR), :]

    q = [window(0, g, 0) for g in range(NG)]
    logits = []
    for w in range(WIN):
        acc = q[0] * window(1, 0, w)
        for g in range(1, NG):
            acc = acc + q[g] * window(1, g, w)
        logits.append(acc)
    for sh in (1, 16):
        low = (lane & sh) == 0
        logits = [x + jnp.where(low, pltpu.roll(x, 128 - sh, 1), pltpu.roll(x, sh, 1)) for x in logits]
    if masked:
        pos = lax.broadcasted_iota(jnp.int32, (AR, 128), 0) + r
        logits = [jnp.where(pos >= DIL * w, x, -1e9 / scale) if w else x for w, x in enumerate(logits)]
    m = logits[0]
    for w in range(1, WIN):
        m = jnp.maximum(m, logits[w])
    e = [jnp.exp2((l - m) * (scale * LOG2E)) for l in logits]
    den = e[0]
    for w in range(1, WIN):
        den = den + e[w]
    inv = 1.0 / den
    p = [x * inv for x in e]
    for g in range(NG):
        acc = p[0] * window(2, g, 0)
        for w in range(1, WIN):
            acc = acc + p[w] * window(2, g, w)
        o_s[pl.ds(r, AR), g * 128:(g + 1) * 128] = acc.astype(BF16)


def _kernel(x_hbm, c_hbm, wqkv_hbm, wo_hbm, wg_hbm, wu_hbm, wd_hbm, wmod_hbm, out_ref,
            x_s, c_s, wmod_s, wqkv_s, wo_raw, wo_s, wg_s, wu_s, wd_s, mod_s,
            qkv0_s, qkv_s, h_s, h1_s, o_s, x1_s, h2_s, act_s, sems, qsems, xsems):
    t = pl.program_id(0)
    first = t == 0

    def mod_copy(i):
        return pltpu.make_async_copy(wmod_hbm.at[:, pl.ds(pl.multiple_of(i * D, D), D)], wmod_s.at[i], sems.at[i])

    def qkv_copy(p):
        rs = pl.ds(pl.multiple_of((p % QP) * (D // QP), D // QP), D // QP)
        return pltpu.make_async_copy(wqkv_hbm.at[rs, pl.ds(pl.multiple_of((p // QP) * D, D), D)],
                                     wqkv_s.at[p // QP, rs], qsems.at[p])

    def x_copy(i):
        return pltpu.make_async_copy(x_hbm.at[pl.ds(pl.multiple_of(i * TM, TM), TM)], x_s.at[i], xsems.at[i])

    def c_copy():
        return pltpu.make_async_copy(c_hbm, c_s, sems.at[6])

    def wo_copies():
        return [pltpu.make_async_copy(wo_hbm.at[:, pl.ds(g * 128, 128)], wo_raw.at[g], sems.at[9])
                for g in range(NG)]

    def gate_copy(f):
        return pltpu.make_async_copy(wg_hbm.at[:, pl.ds(pl.multiple_of(f * FC, FC), FC)], wg_s.at[f], sems.at[10 + f])

    def up_copy(f):
        return pltpu.make_async_copy(wu_hbm.at[:, pl.ds(pl.multiple_of(f * FC, FC), FC)], wu_s.at[f], sems.at[10 + NF + f])

    def down_copy(n):
        return pltpu.make_async_copy(wd_hbm.at[:, pl.ds(n * NC, NC)], wd_s.at[n], sems.at[10 + 2 * NF + n])

    def compute_mod(i):
        cc = c_s[...].astype(F32)
        sc = jnp.broadcast_to(cc * jax.nn.sigmoid(cc), (16, D)).astype(BF16)
        mod_s[i] = jnp.dot(sc, wmod_s[i], preferred_element_type=F32)[0:8]

    def modulated_ln(x, shift, scale):
        return (_layernorm(x) * (1.0 + mod_s[scale, 0:1, :]) + mod_s[shift, 0:1, :]).astype(BF16)

    def norm1(tile, dst, rs):
        dst[rs, :] = modulated_ln(x_s[tile, rs, :].astype(F32), 0, 1)

    def norm2(rs):
        h2_s[rs, :] = modulated_ln(x1_s[rs, :], 3, 4)

    def row_loop(rows, fn):
        def body(i, carry):
            fn(pl.ds(pl.multiple_of(i * rows, rows), rows))
            return carry

        lax.fori_loop(0, TM // rows, body, 0)

    def part(i, n):
        rows = -(-TM // (n * 16)) * 16
        return pl.ds(pl.multiple_of(jnp.minimum(i * rows, TM - rows), 16), rows)

    def attention_part(src, s0, i, n):
        per = -(-(TM // AR) // n)
        for b in range(per):
            blk = jnp.minimum(i * per + b, TM // AR - 1)
            _attention_block(s0, pl.multiple_of(blk * AR, AR), src, o_s, src is qkv0_s)

    def qkv_loop(src, dst, s0, pieces, copies, ride_along):
        def body(i, carry):
            copies(i)
            y = None
            for k in range(pieces):
                ks = slice(k * (D // pieces), (k + 1) * (D // pieces))
                yk = jnp.dot(src[:, ks], wqkv_s[i, ks, :], preferred_element_type=F32)
                y = yk if k == 0 else y + yk
                ride_along(i, k)
            rs = pl.ds(pl.multiple_of(HALO + s0, 8), TM)
            for g in range(NG):
                dst[i, g, rs, :] = y[:, g * 128:(g + 1) * 128]
            return carry

        lax.fori_loop(0, 3, body, 0)

    @pl.when(first)
    def _():
        for p in range(QP):
            qkv_copy(p).start()
        c_copy().start()
        qkv0_s[1:3, :, 0:HALO, :] = jnp.zeros((2, NG, HALO, 128), F32)

        def perm_body(p, carry):
            qkv_copy(p).wait()
            pl.when(p == 0)(mod_copy(0).start)
            pl.when(p == 2)(x_copy(0).start)
            pl.when(p == 3)(mod_copy(1).start)
            rows = D // QP
            _permute_columns(wqkv_s.at[0], pl.ds(pl.multiple_of(p * rows, rows), rows), True)
            return carry

        lax.fori_loop(0, QP, perm_body, 0)
        c_copy().wait()

        def mod_body(i, carry):
            mod_copy(i).wait()

            @pl.when(i == 1)
            def _():
                for p in range(QP, 2 * QP):
                    qkv_copy(p).start()
                x_copy(1).start()

            compute_mod(i)
            return carry

        lax.fori_loop(0, 2, mod_body, 0)
        x_copy(0).wait()
        row_loop(128, lambda rs: norm1(0, h_s, rs))
        x_copy(1).wait()

        def copies_0(i):
            @pl.when(i == 0)
            def _():
                for p in range(2 * QP, 3 * QP):
                    qkv_copy(p).start()

            @pl.when(i == 1)
            def _():
                for cp in wo_copies():
                    cp.start()

            for j in range(2):
                pl.when(i > 0)(mod_copy(2 * jnp.maximum(i, 1) + j).start)

            @pl.when(i < 2)
            def _():
                for p in range(QP):
                    qkv_copy((i + 1) * QP + p).wait()

        def ride_permute(i, k):
            _permute_columns(wqkv_s.at[i + 1], pl.ds(k * (D // KP), D // KP), False)
            if k == 0:
                norm1(1, h1_s, part(i, 3))

        qkv_loop(h_s, qkv0_s, 0, KP, copies_0, ride_permute)
        qkv_s[1:3, :, 0:HALO, :] = qkv0_s[1:3, :, TM:TM + HALO, :]
        for cp in wo_copies():
            cp.wait()

        def copies_1(i):
            @pl.when(i == 0)
            def _():
                for j in range(2, NT):
                    x_copy(j).start()

            for j in range(2):
                gate_copy(2 * i + j).start()
                up_copy(2 * i + j).start()

        def ride_attention(i, k):
            attention_part(qkv0_s, 0, i, 4)
            for j in range(3):
                _permute_rows(wo_raw, wo_s, jnp.minimum(3 * i + j, NG - 1))

        qkv_loop(h1_s, qkv_s, 0, 1, copies_1, ride_attention)
        gate_copy(NF - 1).start()
        up_copy(NF - 1).start()
        for n in range(D // NC):
            down_copy(n).start()

        def mod_rest(i, carry):
            mod_copy(i).wait()
            compute_mod(i)
            attention_part(qkv0_s, 0, 10 + i, 16)
            return carry

        lax.fori_loop(2, 6, mod_rest, 0)

    @pl.when(t > 0)
    def _():
        pl.when(t + 1 < NT)(lambda: x_copy(t + 1).wait())

        def gate_up(f, carry):
            @pl.when(t == 1)
            def _():
                gate_copy(f).wait()
                up_copy(f).wait()

            norm1(jnp.minimum(t + 1, NT - 1), h_s, part(f, NF))
            attention_part(qkv_s, (jnp.minimum(t, NT - 1) - 1) * TM, f, NF)
            h2 = h2_s[...]
            g = jnp.dot(h2, wg_s[f], preferred_element_type=F32)
            u = jnp.dot(h2, wu_s[f], preferred_element_type=F32)
            act_s[f] = (g * jax.nn.sigmoid(g) * u).astype(BF16)
            return carry

        lax.fori_loop(0, NF, gate_up, 0)

        def down(n, carry):
            @pl.when(t == 1)
            def _():
                down_copy(n).wait()

            y = None
            for f in range(NF):
                yf = jnp.dot(act_s[f], wd_s[n, f * FC:(f + 1) * FC, :], preferred_element_type=F32)
                y = yf if f == 0 else y + yf
            cs = pl.ds(pl.multiple_of(n * NC, NC), NC)
            out_ref[:, cs] = (x1_s[:, cs] + mod_s[5, 0:1, cs] * y).astype(out_ref.dtype)
            return carry

        lax.fori_loop(0, D // NC, down, 0)

    @pl.when(t < NT)
    def _():
        def proj(rs):
            a = jnp.dot(o_s[rs, :], wo_s[...], preferred_element_type=F32)
            x1_s[rs, :] = x_s[t, rs, :].astype(F32) + mod_s[2, 0:1, :] * a

        row_loop(PR, proj)

    @pl.when(jnp.logical_and(t > 0, t + 1 < NT))
    def _():
        qkv_loop(h_s, qkv_s, t * TM, 1, lambda i: None, lambda i, k: norm2(part(i, 3)))

    @pl.when(jnp.logical_or(first, t + 1 == NT))
    def _():
        row_loop(128, norm2)


@jax.jit
def pallas_adaLN_cond__sliding_local_dilated__swiglu_ffn__prompt_kernel(
    A_x: jax.Array,
    A_wqkv: jax.Array,
    A_wo: jax.Array,
    B_x: jax.Array,
    B_w_gate: jax.Array,
    B_w_up: jax.Array,
    B_w_down: jax.Array,
    c: jax.Array,
    w_mod: jax.Array,
):
    del B_x
    hbm = pl.BlockSpec(memory_space=pl.ANY)
    out = pl.pallas_call(
        _kernel,
        grid=(NT + 1,),
        in_specs=[hbm] * 8,
        out_specs=pl.BlockSpec((TM, D), lambda t: (jnp.maximum(t - 1, 0), 0)),
        out_shape=jax.ShapeDtypeStruct((S, D), A_x.dtype),
        scratch_shapes=[
            pltpu.VMEM((NT, TM, D), BF16),
            pltpu.VMEM((1, D), BF16),
            pltpu.VMEM((6, D, D), BF16),
            pltpu.VMEM((4, D, D), BF16),
            pltpu.VMEM((NG, D, 128), BF16),
            pltpu.VMEM((D, D), BF16),
            pltpu.VMEM((NF, D, FC), BF16),
            pltpu.VMEM((NF, D, FC), BF16),
            pltpu.VMEM((D // NC, F, NC), BF16),
            pltpu.VMEM((6, 8, D), F32),
            pltpu.VMEM((3, NG, HALO + TM, 128), F32),
            pltpu.VMEM((3, NG, HALO + S - TM, 128), F32),
            pltpu.VMEM((TM, D), BF16),
            pltpu.VMEM((TM, D), BF16),
            pltpu.VMEM((TM, D), BF16),
            pltpu.VMEM((TM, D), F32),
            pltpu.VMEM((TM, D), BF16),
            pltpu.VMEM((NF, TM, FC), BF16),
            pltpu.SemaphoreType.DMA((10 + 2 * NF + D // NC,)),
            pltpu.SemaphoreType.DMA((3 * QP,)),
            pltpu.SemaphoreType.DMA((NT,)),
        ],
        compiler_params=pltpu.CompilerParams(
            dimension_semantics=("arbitrary",),
            flags={'XLA_TPU_EVENLY_DISTRIBUTE_CRITICAL_NODES': True},
            vmem_limit_bytes=112 * 1024 * 1024,
        ),
    )(A_x.reshape(S, D), c, A_wqkv, A_wo, B_w_gate, B_w_up, B_w_down, w_mod)
    return out.reshape(A_x.shape)
```

```python
import jax
import jax.numpy as jnp
from jax import lax
from jax.experimental import pallas as pl
from jax.experimental.pallas import tpu as pltpu

S, D, F = 2048, 1024, 3584
H, DH, WIN, DIL = 32, 32, 8, 2
TM = 512
NT = S // TM
FC = 896
NF = F // FC
NC = 256
HALO = 16
AR = 16
PR = 512
KP = 8
ATT_G, ATT_D = 6, 2
ATT_A = 11
QP = 4
NG = D // 128
EPS = 1e-5
LOG2E = 1.4426950408889634
F32, BF16 = jnp.float32, jnp.bfloat16


def _layernorm(x):
    m = jnp.mean(x, axis=-1, keepdims=True)
    xc = x - m
    v = jnp.mean(xc * xc, axis=-1, keepdims=True)
    return xc * lax.rsqrt(v + EPS)


def _permute_columns(w_ref, rs, on_mxu):
    shift = (lax.broadcasted_iota(jnp.int32, (128, 128), 1)
             - lax.broadcasted_iota(jnp.int32, (128, 128), 0)) & 127

    def roll(x, n):
        if n == 0:
            return x
        if not on_mxu:
            return pltpu.roll(x, n % 128, 1)
        rot = (shift == n % 128).astype(F32).astype(BF16)
        y = jnp.dot(pltpu.bitcast(x, BF16), rot, preferred_element_type=F32)
        return pltpu.bitcast(y.astype(BF16), jnp.uint32)

    cols = [roll(pltpu.bitcast(w_ref[rs, g * 128:(g + 1) * 128], jnp.uint32), 2 * g) for g in range(NG)]
    cols = [cols[-g % NG] for g in range(NG)]
    field = lax.broadcasted_iota(jnp.int32, cols[0].shape, 1) >> 1
    for b in (1, 2, 4):
        bit = (field & b) != 0
        cols = [jnp.where(bit, cols[(g - b) % NG], cols[g]) for g in range(NG)]
    for g in range(NG):
        w_ref[rs, g * 128:(g + 1) * 128] = pltpu.bitcast(roll(cols[g], -2 * g), BF16)


def _permute_rows(src_ref, dst_ref, g):
    cs = pl.ds(pl.multiple_of(g * 128, 128), 128)
    for j in range(8):
        for m in range(8):
            pairs = src_ref[g, pl.ds(m * 8 + j, 8, stride=64), :]
            dst_ref[j * 128 + m * 16:j * 128 + m * 16 + 16, cs] = pltpu.bitcast(pairs, BF16)


def _attention_block(s0, r, qkv_s, o_s, masked):
    scale = DH ** -0.5
    lane = lax.broadcasted_iota(jnp.int32, (AR, 128), 1)

    def window(which, g, w):
        return qkv_s[which, g, pl.ds(s0 + r + (HALO - DIL * w), AR), :]

    q = [window(0, g, 0) for g in range(NG)]
    logits = []
    for w in range(WIN):
        acc = q[0] * window(1, 0, w)
        for g in range(1, NG):
            acc = acc + q[g] * window(1, g, w)
        logits.append(acc)
    for sh in (1, 16):
        low = (lane & sh) == 0
        logits = [x + jnp.where(low, pltpu.roll(x, 128 - sh, 1), pltpu.roll(x, sh, 1)) for x in logits]
    if masked:
        pos = lax.broadcasted_iota(jnp.int32, (AR, 128), 0) + r
        logits = [jnp.where(pos >= DIL * w, x, -1e9 / scale) if w else x for w, x in enumerate(logits)]
    m = logits[0]
    for w in range(1, WIN):
        m = jnp.maximum(m, logits[w])
    e = [jnp.exp2((l - m) * (scale * LOG2E)) for l in logits]
    den = e[0]
    for w in range(1, WIN):
        den = den + e[w]
    inv = 1.0 / den
    p = [x * inv for x in e]
    for g in range(NG):
        acc = p[0] * window(2, g, 0)
        for w in range(1, WIN):
            acc = acc + p[w] * window(2, g, w)
        o_s[pl.ds(r, AR), g * 128:(g + 1) * 128] = acc.astype(BF16)


def _kernel(x_hbm, c_hbm, wqkv_hbm, wo_hbm, wg_hbm, wu_hbm, wd_hbm, wmod_hbm, out_hbm,
            x_s, c_s, wmod_s, wqkv_s, wo_raw, wo_s, wg_s, wu_s, wd_s, mod_s,
            qkv0_s, qkv_s, h_s, h1_s, o_s, x1_s, h2_s, act_s, out_s, sems, qsems, xsems, osems):
    t = pl.program_id(0)
    first = t == 0

    def mod_copy(i):
        return pltpu.make_async_copy(wmod_hbm.at[:, pl.ds(pl.multiple_of(i * D, D), D)], wmod_s.at[i], sems.at[i])

    def qkv_copy(p):
        rs = pl.ds(pl.multiple_of((p % QP) * (D // QP), D // QP), D // QP)
        return pltpu.make_async_copy(wqkv_hbm.at[rs, pl.ds(pl.multiple_of((p // QP) * D, D), D)],
                                     wqkv_s.at[p // QP, rs], qsems.at[p])

    def x_copy(i):
        return pltpu.make_async_copy(x_hbm.at[pl.ds(pl.multiple_of(i * TM, TM), TM)], x_s.at[i], xsems.at[i])

    def c_copy():
        return pltpu.make_async_copy(c_hbm, c_s, sems.at[6])

    def wo_copies():
        return [pltpu.make_async_copy(wo_hbm.at[:, pl.ds(g * 128, 128)], wo_raw.bitcast(BF16).at[g], sems.at[9])
                for g in range(NG)]

    def gate_copy(f):
        return pltpu.make_async_copy(wg_hbm.at[:, pl.ds(pl.multiple_of(f * FC, FC), FC)], wg_s.at[f], sems.at[10 + f])

    def up_copy(f):
        return pltpu.make_async_copy(wu_hbm.at[:, pl.ds(pl.multiple_of(f * FC, FC), FC)], wu_s.at[f], sems.at[10 + NF + f])

    def down_copy(n):
        return pltpu.make_async_copy(wd_hbm.at[:, pl.ds(pl.multiple_of(n * NC, NC), NC)], wd_s.at[n], sems.at[10 + 2 * NF + n])

    def out_copy(tile, n):
        rows = pl.ds(pl.multiple_of(tile * TM, TM), TM)
        return pltpu.make_async_copy(
            out_s.at[n], out_hbm.at[rows, pl.ds(pl.multiple_of(n * NC, NC), NC)], osems.at[n])

    def compute_mod(i):
        cc = c_s[...].astype(F32)
        sc = jnp.broadcast_to(cc * jax.nn.sigmoid(cc), (16, D)).astype(BF16)
        mod_s[i] = jnp.dot(sc, wmod_s[i], preferred_element_type=F32)[0:8]

    def modulated_ln(x, shift, scale):
        return (_layernorm(x) * (1.0 + mod_s[scale, 0:1, :]) + mod_s[shift, 0:1, :]).astype(BF16)

    def norm1(tile, dst, rs):
        dst[rs, :] = modulated_ln(x_s[tile, rs, :].astype(F32), 0, 1)

    def norm2(rs):
        h2_s[rs, :] = modulated_ln(x1_s[rs, :], 3, 4)

    def row_loop(rows, fn):
        def body(i, carry):
            fn(pl.ds(pl.multiple_of(i * rows, rows), rows))
            return carry

        lax.fori_loop(0, TM // rows, body, 0)

    def part(i, n):
        rows = -(-TM // (n * 16)) * 16
        return pl.ds(pl.multiple_of(jnp.minimum(i * rows, TM - rows), 16), rows)

    def attention_part(src, s0, blk0, count):
        for b in range(count):
            blk = jnp.minimum(blk0 + b, TM // AR - 1)
            _attention_block(s0, pl.multiple_of(blk * AR, AR), src, o_s, src is qkv0_s)

    def qkv_loop(src, dst, s0, pieces, copies, ride_along):
        def body(i, carry):
            copies(i)
            y = None
            for k in range(pieces):
                ks = slice(k * (D // pieces), (k + 1) * (D // pieces))
                yk = jnp.dot(src[:, ks], wqkv_s[i, ks, :], preferred_element_type=F32)
                y = yk if k == 0 else y + yk
                ride_along(i, k)
            rs = pl.ds(pl.multiple_of(HALO + s0, 8), TM)
            for g in range(NG):
                dst[i, g, rs, :] = y[:, g * 128:(g + 1) * 128]
            return carry

        lax.fori_loop(0, 3, body, 0)

    @pl.when(first)
    def _():
        for p in range(QP):
            qkv_copy(p).start()
        c_copy().start()
        qkv0_s[1:3, :, 0:HALO, :] = jnp.zeros((2, NG, HALO, 128), F32)

        def perm_body(p, carry):
            qkv_copy(p).wait()
            pl.when(p == 0)(mod_copy(0).start)
            pl.when(p == 2)(x_copy(0).start)
            pl.when(p == 3)(mod_copy(1).start)
            rows = D // QP
            _permute_columns(wqkv_s.at[0], pl.ds(pl.multiple_of(p * rows, rows), rows), True)
            return carry

        lax.fori_loop(0, QP, perm_body, 0)
        c_copy().wait()

        def mod_body(i, carry):
            mod_copy(i).wait()

            @pl.when(i == 1)
            def _():
                for p in range(QP, 2 * QP):
                    qkv_copy(p).start()

            compute_mod(i)
            return carry

        lax.fori_loop(0, 2, mod_body, 0)
        x_copy(0).wait()
        row_loop(128, lambda rs: norm1(0, h_s, rs))

        def copies_0(i):
            @pl.when(i == 0)
            def _():
                x_copy(1).start()
                for p in range(2 * QP, 3 * QP):
                    qkv_copy(p).start()

            @pl.when(i == 1)
            def _():
                x_copy(1).wait()
                for cp in wo_copies():
                    cp.start()

            for j in range(2):
                pl.when(i > 0)(mod_copy(2 * jnp.maximum(i, 1) + j).start)

            @pl.when(i < 2)
            def _():
                for p in range(QP):
                    qkv_copy((i + 1) * QP + p).wait()

        def ride_permute(i, k):
            _permute_columns(wqkv_s.at[i + 1], pl.ds(k * (D // KP), D // KP), False)
            if k == 0:
                norm1(jnp.minimum(i, 1), h1_s, part(jnp.maximum(i, 1) - 1, 2))

        qkv_loop(h_s, qkv0_s, 0, KP, copies_0, ride_permute)
        qkv_s[1:3, :, 0:HALO, :] = qkv0_s[1:3, :, TM:TM + HALO, :]
        for cp in wo_copies():
            cp.wait()

        def copies_1(i):
            @pl.when(i == 0)
            def _():
                for j in range(2, NT):
                    x_copy(j).start()

            gate_copy(i).start()
            up_copy(i).start()

        def ride_attention(i, k):
            attention_part(qkv0_s, 0, i * ATT_A, ATT_A)

        qkv_loop(h1_s, qkv_s, 0, 1, copies_1, ride_attention)
        gate_copy(NF - 1).start()
        up_copy(NF - 1).start()
        for n in range(D // NC):
            down_copy(n).start()

        def mod_rest(i, carry):
            mod_copy(i).wait()
            compute_mod(i)
            for j in range(2):
                _permute_rows(wo_raw, wo_s, 2 * (i - 2) + j)
            return carry

        lax.fori_loop(2, 6, mod_rest, 0)

    @pl.when(t > 0)
    def _():
        pl.when(t + 1 < NT)(lambda: x_copy(t + 1).wait())

        def gate_up(f, carry):
            @pl.when(t == 1)
            def _():
                gate_copy(f).wait()
                up_copy(f).wait()

            norm1(jnp.minimum(t + 1, NT - 1), h_s, part(f, NF))
            attention_part(qkv_s, (jnp.minimum(t, NT - 1) - 1) * TM, f * ATT_G, ATT_G)
            h2 = h2_s[...]
            g = jnp.dot(h2, wg_s[f], preferred_element_type=F32)
            u = jnp.dot(h2, wu_s[f], preferred_element_type=F32)
            act_s[f] = (g * jax.nn.sigmoid(g) * u).astype(BF16)
            return carry

        lax.fori_loop(0, NF, gate_up, 0)

        def down(n, carry):
            @pl.when(t == 1)
            def _():
                down_copy(n).wait()

            pl.when(t > 1)(lambda: out_copy(t - 2, n).wait())
            attention_part(qkv_s, (jnp.minimum(t, NT - 1) - 1) * TM, NF * ATT_G + n * ATT_D, ATT_D)
            y = None
            for f in range(NF):
                yf = jnp.dot(act_s[f], wd_s[n, f * FC:(f + 1) * FC, :], preferred_element_type=F32)
                y = yf if f == 0 else y + yf
            cs = pl.ds(pl.multiple_of(n * NC, NC), NC)
            out_s[n] = (x1_s[:, cs] + mod_s[5, 0:1, cs] * y).astype(out_s.dtype)
            out_copy(t - 1, n).start()
            return carry

        lax.fori_loop(0, D // NC, down, 0)

    @pl.when(t < NT)
    def _():
        def proj(rs):
            a = jnp.dot(o_s[rs, :], wo_s[...], preferred_element_type=F32)
            x1_s[rs, :] = x_s[t, rs, :].astype(F32) + mod_s[2, 0:1, :] * a

        row_loop(PR, proj)

    @pl.when(jnp.logical_and(t > 0, t + 1 < NT))
    def _():
        qkv_loop(h_s, qkv_s, t * TM, 1, lambda i: None, lambda i, k: norm2(part(i, 3)))

    @pl.when(jnp.logical_or(first, t + 1 == NT))
    def _():
        row_loop(128, norm2)

    @pl.when(t == NT)
    def _():
        for n in range(D // NC):
            out_copy(NT - 1, n).wait()


@jax.jit
def pallas_adaLN_cond__sliding_local_dilated__swiglu_ffn__prompt_kernel(
    A_x: jax.Array,
    A_wqkv: jax.Array,
    A_wo: jax.Array,
    B_x: jax.Array,
    B_w_gate: jax.Array,
    B_w_up: jax.Array,
    B_w_down: jax.Array,
    c: jax.Array,
    w_mod: jax.Array,
):
    del B_x
    hbm = pl.BlockSpec(memory_space=pl.ANY)
    out = pl.pallas_call(
        _kernel,
        grid=(NT + 1,),
        in_specs=[hbm] * 8,
        out_specs=hbm,
        out_shape=jax.ShapeDtypeStruct((S, D), A_x.dtype),
        scratch_shapes=[
            pltpu.VMEM((NT, TM, D), BF16),
            pltpu.VMEM((1, D), BF16),
            pltpu.VMEM((6, D, D), BF16),
            pltpu.VMEM((4, D, D), BF16),
            pltpu.VMEM((NG, D // 2, 128), jnp.uint32),
            pltpu.VMEM((D, D), BF16),
            pltpu.VMEM((NF, D, FC), BF16),
            pltpu.VMEM((NF, D, FC), BF16),
            pltpu.VMEM((D // NC, F, NC), BF16),
            pltpu.VMEM((6, 8, D), F32),
            pltpu.VMEM((3, NG, HALO + TM, 128), F32),
            pltpu.VMEM((3, NG, HALO + S - TM, 128), F32),
            pltpu.VMEM((TM, D), BF16),
            pltpu.VMEM((TM, D), BF16),
            pltpu.VMEM((TM, D), BF16),
            pltpu.VMEM((TM, D), F32),
            pltpu.VMEM((TM, D), BF16),
            pltpu.VMEM((NF, TM, FC), BF16),
            pltpu.VMEM((D // NC, TM, NC), A_x.dtype),
            pltpu.SemaphoreType.DMA((10 + 2 * NF + D // NC,)),
            pltpu.SemaphoreType.DMA((3 * QP,)),
            pltpu.SemaphoreType.DMA((NT,)),
            pltpu.SemaphoreType.DMA((D // NC,)),
        ],
        compiler_params=pltpu.CompilerParams(
            dimension_semantics=("arbitrary",),
            flags={'XLA_TPU_EVENLY_DISTRIBUTE_CRITICAL_NODES': True},
            vmem_limit_bytes=112 * 1024 * 1024,
        ),
    )(A_x.reshape(S, D), c, A_wqkv, A_wo, B_w_gate, B_w_up, B_w_down, w_mod)
    return out.reshape(A_x.shape)
```

```python
import jax
import jax.numpy as jnp
from jax import lax
from jax.experimental import pallas as pl
from jax.experimental.pallas import tpu as pltpu

S, D, F = 2048, 1024, 3584
H, DH, WIN, DIL = 32, 32, 8, 2
TM = 512
NT = S // TM
FC = 896
NF = F // FC
NC = 256
HALO = 16
AR = 16
KP = 8
QP = 4
NG = D // 128
EPS = 1e-5
LOG2E = 1.4426950408889634
F32, BF16 = jnp.float32, jnp.bfloat16


def _layernorm(x):
    m = jnp.mean(x, axis=-1, keepdims=True)
    xc = x - m
    v = jnp.mean(xc * xc, axis=-1, keepdims=True)
    return xc * lax.rsqrt(v + EPS)


def _permute_columns(w_ref, rs, on_mxu):
    shift = (lax.broadcasted_iota(jnp.int32, (128, 128), 1)
             - lax.broadcasted_iota(jnp.int32, (128, 128), 0)) & 127

    def roll(x, n):
        if n == 0:
            return x
        if not on_mxu:
            return pltpu.roll(x, n % 128, 1)
        rot = (shift == n % 128).astype(F32).astype(BF16)
        y = jnp.dot(pltpu.bitcast(x, BF16), rot, preferred_element_type=F32)
        return pltpu.bitcast(y.astype(BF16), jnp.uint32)

    cols = [roll(pltpu.bitcast(w_ref[rs, g * 128:(g + 1) * 128], jnp.uint32), 2 * g) for g in range(NG)]
    cols = [cols[-g % NG] for g in range(NG)]
    field = lax.broadcasted_iota(jnp.int32, cols[0].shape, 1) >> 1
    for b in (1, 2, 4):
        bit = (field & b) != 0
        cols = [jnp.where(bit, cols[(g - b) % NG], cols[g]) for g in range(NG)]
    for g in range(NG):
        w_ref[rs, g * 128:(g + 1) * 128] = pltpu.bitcast(roll(cols[g], -2 * g), BF16)


def _permute_rows(src_ref, dst_ref, g):
    cs = pl.ds(pl.multiple_of(g * 128, 128), 128)
    for j in range(8):
        for m in range(8):
            pairs = src_ref[g, pl.ds(m * 8 + j, 8, stride=64), :]
            dst_ref[j * 128 + m * 16:j * 128 + m * 16 + 16, cs] = pltpu.bitcast(pairs, BF16)


def _attention_block(s0, r, qkv_s, o_s, masked):
    scale = DH ** -0.5
    lane = lax.broadcasted_iota(jnp.int32, (AR, 128), 1)

    def window(which, g, w):
        return qkv_s[which, g, pl.ds(s0 + r + (HALO - DIL * w), AR), :]

    q = [window(0, g, 0) for g in range(NG)]
    logits = []
    for w in range(WIN):
        acc = q[0] * window(1, 0, w)
        for g in range(1, NG):
            acc = acc + q[g] * window(1, g, w)
        logits.append(acc)
    for sh in (1, 16):
        low = (lane & sh) == 0
        logits = [x + jnp.where(low, pltpu.roll(x, 128 - sh, 1), pltpu.roll(x, sh, 1)) for x in logits]
    if masked:
        pos = lax.broadcasted_iota(jnp.int32, (AR, 128), 0) + r
        logits = [jnp.where(pos >= DIL * w, x, -1e9 / scale) if w else x for w, x in enumerate(logits)]
    m = logits[0]
    for w in range(1, WIN):
        m = jnp.maximum(m, logits[w])
    e = [jnp.exp2((l - m) * (scale * LOG2E)) for l in logits]
    den = e[0]
    for w in range(1, WIN):
        den = den + e[w]
    inv = 1.0 / den
    p = [x * inv for x in e]
    for g in range(NG):
        acc = p[0] * window(2, g, 0)
        for w in range(1, WIN):
            acc = acc + p[w] * window(2, g, w)
        o_s[pl.ds(r, AR), g * 128:(g + 1) * 128] = acc.astype(BF16)


def _kernel(x_hbm, c_hbm, wqkv_hbm, wo_hbm, wg_hbm, wu_hbm, wd_hbm, wmod_hbm, out_hbm,
            x_s, c_s, wmod_s, wqkv_s, wo_raw, wo_s, wg_s, wu_s, wd_s, mod_s,
            qkv0_s, qkv_s, h_s, h1_s, o_s, x1_s, h2_s, act_s, out_s, sems, qsems, xsems, osems):
    t = pl.program_id(0)
    first = t == 0

    def mod_copy(i):
        return pltpu.make_async_copy(wmod_hbm.at[:, pl.ds(pl.multiple_of(i * D, D), D)], wmod_s.at[i], sems.at[i])

    def qkv_copy(p):
        rs = pl.ds(pl.multiple_of((p % QP) * (D // QP), D // QP), D // QP)
        return pltpu.make_async_copy(wqkv_hbm.at[rs, pl.ds(pl.multiple_of((p // QP) * D, D), D)],
                                     wqkv_s.at[p // QP, rs], qsems.at[p])

    def x_copy(i):
        return pltpu.make_async_copy(x_hbm.at[pl.ds(pl.multiple_of(i * TM, TM), TM)], x_s.at[i], xsems.at[i])

    def c_copy():
        return pltpu.make_async_copy(c_hbm, c_s, sems.at[6])

    def wo_copies():
        return [pltpu.make_async_copy(wo_hbm.at[:, pl.ds(g * 128, 128)], wo_raw.bitcast(BF16).at[g], sems.at[9])
                for g in range(NG)]

    def gate_copy(f):
        return pltpu.make_async_copy(wg_hbm.at[:, pl.ds(pl.multiple_of(f * FC, FC), FC)], wg_s.at[f], sems.at[10 + f])

    def up_copy(f):
        return pltpu.make_async_copy(wu_hbm.at[:, pl.ds(pl.multiple_of(f * FC, FC), FC)], wu_s.at[f], sems.at[10 + NF + f])

    def down_copy(n):
        return pltpu.make_async_copy(wd_hbm.at[:, pl.ds(pl.multiple_of(n * NC, NC), NC)], wd_s.at[n], sems.at[10 + 2 * NF + n])

    def out_copy(tile, n):
        rows = pl.ds(pl.multiple_of(tile * TM, TM), TM)
        return pltpu.make_async_copy(
            out_s.at[n], out_hbm.at[rows, pl.ds(pl.multiple_of(n * NC, NC), NC)], osems.at[n])

    def compute_mod(i):
        cc = c_s[...].astype(F32)
        sc = jnp.broadcast_to(cc * jax.nn.sigmoid(cc), (16, D)).astype(BF16)
        mod_s[i] = jnp.dot(sc, wmod_s[i], preferred_element_type=F32)[0:8]

    def mod(i):
        return mod_s[i, 0:1, :]

    def modulated_ln(x, shift, scale):
        return (_layernorm(x) * (1.0 + mod(scale)) + mod(shift)).astype(BF16)

    def norm1(tile, dst, rs):
        dst[rs, :] = modulated_ln(x_s[tile, rs, :].astype(F32), 0, 1)

    def norm2(slot, rs):
        h2_s[rs, :] = modulated_ln(x1_s[slot, rs, :], 3, 4)

    def row_loop(rows, fn):
        def body(i, carry):
            fn(pl.ds(pl.multiple_of(i * rows, rows), rows))
            return carry

        lax.fori_loop(0, TM // rows, body, 0)

    def part(i, n):
        rows = -(-TM // (n * 16)) * 16
        return pl.ds(pl.multiple_of(jnp.minimum(i * rows, TM - rows), 16), rows)

    def attention_part(src, s0, i, n):
        per = -(-(TM // AR) // n)
        for b in range(per):
            blk = jnp.minimum(i * per + b, TM // AR - 1)
            _attention_block(s0, pl.multiple_of(blk * AR, AR), src, o_s, src is qkv0_s)

    def qkv_loop(src, dst, s0, pieces, copies, ride_along):
        def body(i, carry):
            copies(i)
            y = None
            for k in range(pieces):
                ks = slice(k * (D // pieces), (k + 1) * (D // pieces))
                yk = jnp.dot(src[:, ks], wqkv_s[i, ks, :], preferred_element_type=F32)
                y = yk if k == 0 else y + yk
                ride_along(i, k)
            rs = pl.ds(pl.multiple_of(HALO + s0, 8), TM)
            for g in range(NG):
                dst[i, g, rs, :] = y[:, g * 128:(g + 1) * 128]
            return carry

        lax.fori_loop(0, 3, body, 0)

    @pl.when(first)
    def _():
        for p in range(QP):
            qkv_copy(p).start()
        c_copy().start()
        qkv0_s[1:3, :, 0:HALO, :] = jnp.zeros((2, NG, HALO, 128), F32)

        def perm_body(p, carry):
            qkv_copy(p).wait()
            pl.when(p == 0)(mod_copy(0).start)
            pl.when(p == 2)(x_copy(0).start)
            pl.when(p == 3)(mod_copy(1).start)
            rows = D // QP
            _permute_columns(wqkv_s.at[0], pl.ds(pl.multiple_of(p * rows, rows), rows), True)
            return carry

        lax.fori_loop(0, QP, perm_body, 0)
        c_copy().wait()

        def mod_body(i, carry):
            mod_copy(i).wait()

            @pl.when(i == 1)
            def _():
                for p in range(QP, 2 * QP):
                    qkv_copy(p).start()

            compute_mod(i)
            return carry

        lax.fori_loop(0, 2, mod_body, 0)
        x_copy(0).wait()
        row_loop(128, lambda rs: norm1(0, h_s, rs))

        def copies_0(i):
            @pl.when(i == 0)
            def _():
                x_copy(1).start()
                for p in range(2 * QP, 3 * QP):
                    qkv_copy(p).start()

            @pl.when(i == 1)
            def _():
                x_copy(1).wait()
                for cp in wo_copies():
                    cp.start()

            for j in range(2):
                pl.when(i > 0)(mod_copy(2 * jnp.maximum(i, 1) + j).start)

            @pl.when(i < 2)
            def _():
                for p in range(QP):
                    qkv_copy((i + 1) * QP + p).wait()

        def ride_permute(i, k):
            _permute_columns(wqkv_s.at[i + 1], pl.ds(k * (D // KP), D // KP), False)
            norm1(jnp.minimum(i, 1), h1_s, part((jnp.maximum(i, 1) - 1) * KP + k, 2 * KP))

        qkv_loop(h_s, qkv0_s, 0, KP, copies_0, ride_permute)
        qkv_s[1:3, :, 0:HALO, :] = qkv0_s[1:3, :, TM:TM + HALO, :]
        for cp in wo_copies():
            cp.wait()

        def copies_1(i):
            @pl.when(i == 0)
            def _():
                for j in range(2, NT):
                    x_copy(j).start()

            gate_copy(i).start()
            up_copy(i).start()

        def ride_attention(i, k):
            attention_part(qkv0_s, 0, i, 3)

        qkv_loop(h1_s, qkv_s, 0, 1, copies_1, ride_attention)
        gate_copy(NF - 1).start()
        up_copy(NF - 1).start()
        for n in range(D // NC):
            down_copy(n).start()

        def mod_rest(i, carry):
            mod_copy(i).wait()
            compute_mod(i)
            for j in range(2):
                _permute_rows(wo_raw, wo_s, 2 * (i - 2) + j)
            return carry

        lax.fori_loop(2, 6, mod_rest, 0)

    @pl.when(t > 0)
    def _():
        pl.when(t + 1 < NT)(lambda: x_copy(t + 1).wait())

        def gate_up(f, carry):
            @pl.when(t == 1)
            def _():
                gate_copy(f).wait()
                up_copy(f).wait()

            norm1(jnp.minimum(t + 1, NT - 1), h_s, part(f, NF))
            attention_part(qkv_s, (jnp.minimum(t, NT - 1) - 1) * TM, f, NF)
            h2 = h2_s[...]
            g = jnp.dot(h2, wg_s[f], preferred_element_type=F32)
            u = jnp.dot(h2, wu_s[f], preferred_element_type=F32)
            hg = 0.5 * g
            act_s[f] = ((hg + hg * jnp.tanh(hg)) * u).astype(BF16)
            return carry

        lax.fori_loop(0, NF, gate_up, 0)

    @pl.when(t < NT)
    def _():
        a = jnp.dot(o_s[...], wo_s[...], preferred_element_type=F32)
        x1_s[t % 2] = x_s[t].astype(F32) + mod(2) * a

    @pl.when(first)
    def _():
        row_loop(128, lambda rs: norm2(0, rs))

    @pl.when(t > 0)
    def _():
        def down(n, carry):
            @pl.when(t == 1)
            def _():
                down_copy(n).wait()

            pl.when(t > 1)(lambda: out_copy(t - 2, n).wait())
            norm2(jnp.minimum(t, NT - 1) % 2, part(n, D // NC))
            y = None
            for f in range(NF):
                yf = jnp.dot(act_s[f], wd_s[n, f * FC:(f + 1) * FC, :], preferred_element_type=F32)
                y = yf if f == 0 else y + yf
            cs = pl.ds(pl.multiple_of(n * NC, NC), NC)
            out_s[n] = (x1_s[1 - t % 2, :, cs] + mod_s[5, 0:1, cs] * y).astype(out_s.dtype)
            out_copy(t - 1, n).start()
            return carry

        lax.fori_loop(0, D // NC, down, 0)

    @pl.when(jnp.logical_and(t > 0, t + 1 < NT))
    def _():
        qkv_loop(h_s, qkv_s, t * TM, 1, lambda i: None, lambda i, k: None)

    @pl.when(t == NT)
    def _():
        for n in range(D // NC):
            out_copy(NT - 1, n).wait()


@jax.jit
def pallas_adaLN_cond__sliding_local_dilated__swiglu_ffn__prompt_kernel(
    A_x: jax.Array,
    A_wqkv: jax.Array,
    A_wo: jax.Array,
    B_x: jax.Array,
    B_w_gate: jax.Array,
    B_w_up: jax.Array,
    B_w_down: jax.Array,
    c: jax.Array,
    w_mod: jax.Array,
):
    del B_x
    hbm = pl.BlockSpec(memory_space=pl.ANY)
    out = pl.pallas_call(
        _kernel,
        grid=(NT + 1,),
        in_specs=[hbm] * 8,
        out_specs=hbm,
        out_shape=jax.ShapeDtypeStruct((S, D), A_x.dtype),
        scratch_shapes=[
            pltpu.VMEM((NT, TM, D), BF16),
            pltpu.VMEM((1, D), BF16),
            pltpu.VMEM((6, D, D), BF16),
            pltpu.VMEM((4, D, D), BF16),
            pltpu.VMEM((NG, D // 2, 128), jnp.uint32),
            pltpu.VMEM((D, D), BF16),
            pltpu.VMEM((NF, D, FC), BF16),
            pltpu.VMEM((NF, D, FC), BF16),
            pltpu.VMEM((D // NC, F, NC), BF16),
            pltpu.VMEM((6, 8, D), F32),
            pltpu.VMEM((3, NG, HALO + TM, 128), F32),
            pltpu.VMEM((3, NG, HALO + S - TM, 128), F32),
            pltpu.VMEM((TM, D), BF16),
            pltpu.VMEM((TM, D), BF16),
            pltpu.VMEM((TM, D), BF16),
            pltpu.VMEM((2, TM, D), F32),
            pltpu.VMEM((TM, D), BF16),
            pltpu.VMEM((NF, TM, FC), BF16),
            pltpu.VMEM((D // NC, TM, NC), A_x.dtype),
            pltpu.SemaphoreType.DMA((10 + 2 * NF + D // NC,)),
            pltpu.SemaphoreType.DMA((3 * QP,)),
            pltpu.SemaphoreType.DMA((NT,)),
            pltpu.SemaphoreType.DMA((D // NC,)),
        ],
        compiler_params=pltpu.CompilerParams(
            dimension_semantics=("arbitrary",),
            flags={'XLA_TPU_EVENLY_DISTRIBUTE_CRITICAL_NODES': True},
            vmem_limit_bytes=112 * 1024 * 1024,
        ),
    )(A_x.reshape(S, D), c, A_wqkv, A_wo, B_w_gate, B_w_up, B_w_down, w_mod)
    return out.reshape(A_x.shape)
```

```python
import jax
import jax.numpy as jnp
from jax import lax
from jax.experimental import pallas as pl
from jax.experimental.pallas import tpu as pltpu

S, D, F = 2048, 1024, 3584
H, DH, WIN, DIL = 32, 32, 8, 2
TM = 512
NT = S // TM
FC = 896
NF = F // FC
NC = 256
HALO = 16
AR = 16
KP = 8
QP = 4
NG = D // 128
EPS = 1e-5
LOG2E = 1.4426950408889634
F32, BF16 = jnp.float32, jnp.bfloat16


def _layernorm(x):
    m = jnp.mean(x, axis=-1, keepdims=True)
    xc = x - m
    v = jnp.mean(xc * xc, axis=-1, keepdims=True)
    return xc * lax.rsqrt(v + EPS)


def _swap_group_and_field(xs, field, roll):
    xs = [roll(xs[-g % 8], -g % 8) for g in range(8)]
    for b in (1, 2, 4):
        bit = (field & b) != 0
        xs = [jnp.where(bit, xs[(g - b) % 8], xs[g]) for g in range(8)]
    return [roll(x, -g) for g, x in enumerate(xs)]


def _permute_columns(w_ref, rs, on_mxu):
    shift = (lax.broadcasted_iota(jnp.int32, (128, 128), 1)
             - lax.broadcasted_iota(jnp.int32, (128, 128), 0)) & 127

    def roll(x, n):
        if n == 0:
            return x
        if not on_mxu:
            return pltpu.roll(x, 2 * n % 128, 1)
        rot = (shift == 2 * n % 128).astype(F32).astype(BF16)
        y = jnp.dot(pltpu.bitcast(x, BF16), rot, preferred_element_type=F32)
        return pltpu.bitcast(y.astype(BF16), jnp.uint32)

    cols = [pltpu.bitcast(w_ref[rs, g * 128:(g + 1) * 128], jnp.uint32) for g in range(NG)]
    field = lax.broadcasted_iota(jnp.int32, cols[0].shape, 1) >> 1
    for g, x in enumerate(_swap_group_and_field(cols, field, roll)):
        w_ref[rs, g * 128:(g + 1) * 128] = pltpu.bitcast(x, BF16)


def _permute_rows(src_ref, dst_ref, m):
    rows = [pl.ds(pl.multiple_of(c * 128 + m * 16, 16), 16) for c in range(8)]
    field = lax.broadcasted_iota(jnp.int32, (8, 128), 0)
    for g in range(NG):
        cs = slice(g * 128, (g + 1) * 128)
        xs = [pltpu.bitcast(src_ref[r, cs], jnp.uint32) for r in rows]
        xs = _swap_group_and_field(xs, field, lambda x, n: pltpu.roll(x, n % 8, 0) if n else x)
        for r, x in zip(rows, xs):
            dst_ref[r, cs] = pltpu.bitcast(x, BF16)


def _attention_block(s0, r, qkv_s, o_s, masked):
    scale = DH ** -0.5
    lane = lax.broadcasted_iota(jnp.int32, (AR, 128), 1)

    def window(which, g, w):
        return qkv_s[which, g, pl.ds(s0 + r + (HALO - DIL * w), AR), :]

    q = [window(0, g, 0) for g in range(NG)]
    logits = []
    for w in range(WIN):
        acc = q[0] * window(1, 0, w)
        for g in range(1, NG):
            acc = acc + q[g] * window(1, g, w)
        logits.append(acc)
    for sh in (1, 16):
        low = (lane & sh) == 0
        logits = [x + jnp.where(low, pltpu.roll(x, 128 - sh, 1), pltpu.roll(x, sh, 1)) for x in logits]
    if masked:
        pos = lax.broadcasted_iota(jnp.int32, (AR, 128), 0) + r
        logits = [jnp.where(pos >= DIL * w, x, -1e9 / scale) if w else x for w, x in enumerate(logits)]
    m = logits[0]
    for w in range(1, WIN):
        m = jnp.maximum(m, logits[w])
    e = [jnp.exp2((l - m) * (scale * LOG2E)) for l in logits]
    den = e[0]
    for w in range(1, WIN):
        den = den + e[w]
    inv = 1.0 / den
    p = [x * inv for x in e]
    for g in range(NG):
        acc = p[0] * window(2, g, 0)
        for w in range(1, WIN):
            acc = acc + p[w] * window(2, g, w)
        o_s[pl.ds(r, AR), g * 128:(g + 1) * 128] = acc.astype(BF16)


def _kernel(x_hbm, c_hbm, wqkv_hbm, wo_hbm, wg_hbm, wu_hbm, wd_hbm, wmod_hbm, out_hbm,
            x_s, c_s, wmod_s, wqkv_s, wo_raw, wo_s, wg_s, wu_s, wd_s, mod_s,
            qkv0_s, qkv_s, h_s, h1_s, o_s, x1_s, h2_s, act_s, out_s, sems, qsems, xsems, osems):
    t = pl.program_id(0)
    first = t == 0

    def mod_copy(i):
        return pltpu.make_async_copy(wmod_hbm.at[:, pl.ds(pl.multiple_of(i * D, D), D)], wmod_s.at[i], sems.at[i])

    def qkv_copy(p):
        rs = pl.ds(pl.multiple_of((p % QP) * (D // QP), D // QP), D // QP)
        return pltpu.make_async_copy(wqkv_hbm.at[rs, pl.ds(pl.multiple_of((p // QP) * D, D), D)],
                                     wqkv_s.at[p // QP, rs], qsems.at[p])

    def x_copy(i):
        return pltpu.make_async_copy(x_hbm.at[pl.ds(pl.multiple_of(i * TM, TM), TM)], x_s.at[i], xsems.at[i])

    def c_copy():
        return pltpu.make_async_copy(c_hbm, c_s, sems.at[6])

    def wo_copy():
        return pltpu.make_async_copy(wo_hbm, wo_raw, sems.at[9])

    def gate_copy(f):
        return pltpu.make_async_copy(wg_hbm.at[:, pl.ds(pl.multiple_of(f * FC, FC), FC)], wg_s.at[f], sems.at[10 + f])

    def up_copy(f):
        return pltpu.make_async_copy(wu_hbm.at[:, pl.ds(pl.multiple_of(f * FC, FC), FC)], wu_s.at[f], sems.at[10 + NF + f])

    def down_copy(n):
        return pltpu.make_async_copy(wd_hbm.at[:, pl.ds(pl.multiple_of(n * NC, NC), NC)], wd_s.at[n], sems.at[10 + 2 * NF + n])

    def out_copy(tile, n):
        rows = pl.ds(pl.multiple_of(tile * TM, TM), TM)
        return pltpu.make_async_copy(
            out_s.at[n], out_hbm.at[rows, pl.ds(pl.multiple_of(n * NC, NC), NC)], osems.at[n])

    def compute_mod(i):
        cc = c_s[...].astype(F32)
        sc = jnp.broadcast_to(cc * jax.nn.sigmoid(cc), (16, D)).astype(BF16)
        mod_s[i] = jnp.dot(sc, wmod_s[i], preferred_element_type=F32)[0:8]

    def mod(i):
        return mod_s[i, 0:1, :]

    def modulated_ln(x, shift, scale):
        return (_layernorm(x) * (1.0 + mod(scale)) + mod(shift)).astype(BF16)

    def norm1(tile, dst, rs):
        dst[rs, :] = modulated_ln(x_s[tile, rs, :].astype(F32), 0, 1)

    def norm2(slot, rs):
        h2_s[rs, :] = modulated_ln(x1_s[slot, rs, :], 3, 4)

    def row_loop(rows, fn):
        def body(i, carry):
            fn(pl.ds(pl.multiple_of(i * rows, rows), rows))
            return carry

        lax.fori_loop(0, TM // rows, body, 0)

    def part(i, n):
        rows = -(-TM // (n * 16)) * 16
        return pl.ds(pl.multiple_of(jnp.minimum(i * rows, TM - rows), 16), rows)

    def attention_part(src, s0, i, n):
        per = -(-(TM // AR) // n)
        for b in range(per):
            blk = jnp.minimum(i * per + b, TM // AR - 1)
            _attention_block(s0, pl.multiple_of(blk * AR, AR), src, o_s, src is qkv0_s)

    def qkv_loop(src, dst, s0, pieces, copies, ride_along):
        def body(i, carry):
            copies(i)
            y = None
            for k in range(pieces):
                ks = slice(k * (D // pieces), (k + 1) * (D // pieces))
                yk = jnp.dot(src[:, ks], wqkv_s[i, ks, :], preferred_element_type=F32)
                y = yk if k == 0 else y + yk
                ride_along(i, k)
            rs = pl.ds(pl.multiple_of(HALO + s0, 8), TM)
            for g in range(NG):
                dst[i, g, rs, :] = y[:, g * 128:(g + 1) * 128]
            return carry

        lax.fori_loop(0, 3, body, 0)

    @pl.when(first)
    def _():
        for p in range(QP):
            qkv_copy(p).start()
        c_copy().start()
        qkv0_s[1:3, :, 0:HALO, :] = jnp.zeros((2, NG, HALO, 128), F32)

        def perm_body(p, carry):
            qkv_copy(p).wait()
            pl.when(p == 0)(mod_copy(0).start)
            pl.when(p == 2)(x_copy(0).start)
            pl.when(p == 3)(mod_copy(1).start)
            rows = D // QP
            _permute_columns(wqkv_s.at[0], pl.ds(pl.multiple_of(p * rows, rows), rows), True)
            return carry

        lax.fori_loop(0, QP, perm_body, 0)
        c_copy().wait()

        def mod_body(i, carry):
            mod_copy(i).wait()

            @pl.when(i == 1)
            def _():
                for p in range(QP, 2 * QP):
                    qkv_copy(p).start()

            compute_mod(i)
            return carry

        lax.fori_loop(0, 2, mod_body, 0)
        x_copy(0).wait()
        row_loop(128, lambda rs: norm1(0, h_s, rs))

        def copies_0(i):
            @pl.when(i == 0)
            def _():
                x_copy(1).start()
                for p in range(2 * QP, 3 * QP):
                    qkv_copy(p).start()

            @pl.when(i == 1)
            def _():
                x_copy(1).wait()
                wo_copy().start()

            for j in range(2):
                pl.when(i > 0)(mod_copy(2 * jnp.maximum(i, 1) + j).start)

            @pl.when(i < 2)
            def _():
                for p in range(QP):
                    qkv_copy((i + 1) * QP + p).wait()

        def ride_permute(i, k):
            _permute_columns(wqkv_s.at[i + 1], pl.ds(k * (D // KP), D // KP), False)
            norm1(jnp.minimum(i, 1), h1_s, part((jnp.maximum(i, 1) - 1) * KP + k, 2 * KP))

        qkv_loop(h_s, qkv0_s, 0, KP, copies_0, ride_permute)
        qkv_s[1:3, :, 0:HALO, :] = qkv0_s[1:3, :, TM:TM + HALO, :]
        wo_copy().wait()

        def copies_1(i):
            @pl.when(i == 0)
            def _():
                for j in range(2, NT):
                    x_copy(j).start()

            gate_copy(i).start()
            up_copy(i).start()

        def ride_attention(i, k):
            attention_part(qkv0_s, 0, i, 3)
            for j in range(3):
                _permute_rows(wo_raw, wo_s, jnp.minimum(3 * i + j, 7))

        qkv_loop(h1_s, qkv_s, 0, 1, copies_1, ride_attention)
        gate_copy(NF - 1).start()
        up_copy(NF - 1).start()
        for n in range(D // NC):
            down_copy(n).start()

        def mod_rest(i, carry):
            mod_copy(i).wait()
            compute_mod(i)
            return carry

        lax.fori_loop(2, 6, mod_rest, 0)

    @pl.when(t > 0)
    def _():
        pl.when(t + 1 < NT)(lambda: x_copy(t + 1).wait())

        def gate_up(f, carry):
            @pl.when(t == 1)
            def _():
                gate_copy(f).wait()
                up_copy(f).wait()

            norm1(jnp.minimum(t + 1, NT - 1), h_s, part(f, NF))
            attention_part(qkv_s, (jnp.minimum(t, NT - 1) - 1) * TM, f, NF)
            h2 = h2_s[...]
            g = jnp.dot(h2, wg_s[f], preferred_element_type=F32)
            u = jnp.dot(h2, wu_s[f], preferred_element_type=F32)
            hg = 0.5 * g
            act_s[f] = ((hg + hg * jnp.tanh(hg)) * u).astype(BF16)
            return carry

        lax.fori_loop(0, NF, gate_up, 0)

    @pl.when(t < NT)
    def _():
        a = jnp.dot(o_s[...], wo_s[...], preferred_element_type=F32)
        x1_s[t % 2] = x_s[t].astype(F32) + mod(2) * a

    @pl.when(first)
    def _():
        row_loop(128, lambda rs: norm2(0, rs))

    @pl.when(t > 0)
    def _():
        def down(n, carry):
            @pl.when(t == 1)
            def _():
                down_copy(n).wait()

            pl.when(t > 1)(lambda: out_copy(t - 2, n).wait())
            norm2(jnp.minimum(t, NT - 1) % 2, part(n, D // NC))
            y = None
            for f in range(NF):
                yf = jnp.dot(act_s[f], wd_s[n, f * FC:(f + 1) * FC, :], preferred_element_type=F32)
                y = yf if f == 0 else y + yf
            cs = pl.ds(pl.multiple_of(n * NC, NC), NC)
            out_s[n] = (x1_s[1 - t % 2, :, cs] + mod_s[5, 0:1, cs] * y).astype(out_s.dtype)
            out_copy(t - 1, n).start()
            return carry

        lax.fori_loop(0, D // NC, down, 0)

    @pl.when(jnp.logical_and(t > 0, t + 1 < NT))
    def _():
        qkv_loop(h_s, qkv_s, t * TM, 1, lambda i: None, lambda i, k: None)

    @pl.when(t == NT)
    def _():
        for n in range(D // NC):
            out_copy(NT - 1, n).wait()


@jax.jit
def pallas_adaLN_cond__sliding_local_dilated__swiglu_ffn__prompt_kernel(
    A_x: jax.Array,
    A_wqkv: jax.Array,
    A_wo: jax.Array,
    B_x: jax.Array,
    B_w_gate: jax.Array,
    B_w_up: jax.Array,
    B_w_down: jax.Array,
    c: jax.Array,
    w_mod: jax.Array,
):
    del B_x
    hbm = pl.BlockSpec(memory_space=pl.ANY)
    out = pl.pallas_call(
        _kernel,
        grid=(NT + 1,),
        in_specs=[hbm] * 8,
        out_specs=hbm,
        out_shape=jax.ShapeDtypeStruct((S, D), A_x.dtype),
        scratch_shapes=[
            pltpu.VMEM((NT, TM, D), BF16),
            pltpu.VMEM((1, D), BF16),
            pltpu.VMEM((6, D, D), BF16),
            pltpu.VMEM((4, D, D), BF16),
            pltpu.VMEM((D, D), BF16),
            pltpu.VMEM((D, D), BF16),
            pltpu.VMEM((NF, D, FC), BF16),
            pltpu.VMEM((NF, D, FC), BF16),
            pltpu.VMEM((D // NC, F, NC), BF16),
            pltpu.VMEM((6, 8, D), F32),
            pltpu.VMEM((3, NG, HALO + TM, 128), F32),
            pltpu.VMEM((3, NG, HALO + S - TM, 128), F32),
            pltpu.VMEM((TM, D), BF16),
            pltpu.VMEM((TM, D), BF16),
            pltpu.VMEM((TM, D), BF16),
            pltpu.VMEM((2, TM, D), F32),
            pltpu.VMEM((TM, D), BF16),
            pltpu.VMEM((NF, TM, FC), BF16),
            pltpu.VMEM((D // NC, TM, NC), A_x.dtype),
            pltpu.SemaphoreType.DMA((10 + 2 * NF + D // NC,)),
            pltpu.SemaphoreType.DMA((3 * QP,)),
            pltpu.SemaphoreType.DMA((NT,)),
            pltpu.SemaphoreType.DMA((D // NC,)),
        ],
        compiler_params=pltpu.CompilerParams(
            dimension_semantics=("arbitrary",),
            flags={'XLA_TPU_EVENLY_DISTRIBUTE_CRITICAL_NODES': True},
            vmem_limit_bytes=112 * 1024 * 1024,
        ),
    )(A_x.reshape(S, D), c, A_wqkv, A_wo, B_w_gate, B_w_up, B_w_down, w_mod)
    return out.reshape(A_x.shape)
```

```python
import jax
import jax.numpy as jnp
from jax import lax
from jax.experimental import pallas as pl
from jax.experimental.pallas import tpu as pltpu

S, D, F = 2048, 1024, 3584
H, DH, WIN, DIL = 32, 32, 8, 2
TM = 512
NT = S // TM
FC = 896
NF = F // FC
NC = 256
HALO = 16
AR = 16
KP = 8
QP = 4
NG = D // 128
EPS = 1e-5
LOG2E = 1.4426950408889634
F32, BF16 = jnp.float32, jnp.bfloat16


def _layernorm(x):
    m = jnp.mean(x, axis=-1, keepdims=True)
    xc = x - m
    v = jnp.mean(xc * xc, axis=-1, keepdims=True)
    return xc * lax.rsqrt(v + EPS)


def _swap_group_and_field(xs, field, roll):
    xs = [roll(xs[-g % 8], -g % 8) for g in range(8)]
    for b in (1, 2, 4):
        bit = (field & b) != 0
        xs = [jnp.where(bit, xs[(g - b) % 8], xs[g]) for g in range(8)]
    return [roll(x, -g) for g, x in enumerate(xs)]


def _permute_columns(w_ref, rs, on_mxu):
    shift = (lax.broadcasted_iota(jnp.int32, (128, 128), 1)
             - lax.broadcasted_iota(jnp.int32, (128, 128), 0)) & 127

    def roll(x, n):
        if n == 0:
            return x
        if not on_mxu:
            return pltpu.roll(x, 2 * n % 128, 1)
        rot = (shift == 2 * n % 128).astype(F32).astype(BF16)
        y = jnp.dot(pltpu.bitcast(x, BF16), rot, preferred_element_type=F32)
        return pltpu.bitcast(y.astype(BF16), jnp.uint32)

    cols = [pltpu.bitcast(w_ref[rs, g * 128:(g + 1) * 128], jnp.uint32) for g in range(NG)]
    field = lax.broadcasted_iota(jnp.int32, cols[0].shape, 1) >> 1
    for g, x in enumerate(_swap_group_and_field(cols, field, roll)):
        w_ref[rs, g * 128:(g + 1) * 128] = pltpu.bitcast(x, BF16)


def _permute_rows(src_ref, dst_ref, m):
    rows = [pl.ds(pl.multiple_of(c * 128 + m * 16, 16), 16) for c in range(8)]
    field = lax.broadcasted_iota(jnp.int32, (8, 128), 0)
    for g in range(NG):
        cs = slice(g * 128, (g + 1) * 128)
        xs = [pltpu.bitcast(src_ref[r, cs], jnp.uint32) for r in rows]
        xs = _swap_group_and_field(xs, field, lambda x, n: pltpu.roll(x, n % 8, 0) if n else x)
        for r, x in zip(rows, xs):
            dst_ref[r, cs] = pltpu.bitcast(x, BF16)


def _attention_block(s0, r, qkv_s, o_s, masked):
    scale = DH ** -0.5
    lane = lax.broadcasted_iota(jnp.int32, (AR, 128), 1)

    def window(which, g, w):
        return qkv_s[which, g, pl.ds(s0 + r + (HALO - DIL * w), AR), :]

    q = [window(0, g, 0) for g in range(NG)]
    logits = []
    for w in range(WIN):
        acc = q[0] * window(1, 0, w)
        for g in range(1, NG):
            acc = acc + q[g] * window(1, g, w)
        logits.append(acc)
    for sh in (1, 16):
        low = (lane & sh) == 0
        logits = [x + jnp.where(low, pltpu.roll(x, 128 - sh, 1), pltpu.roll(x, sh, 1)) for x in logits]
    if masked:
        pos = lax.broadcasted_iota(jnp.int32, (AR, 128), 0) + r
        logits = [jnp.where(pos >= DIL * w, x, -1e9 / scale) if w else x for w, x in enumerate(logits)]
    m = logits[0]
    for w in range(1, WIN):
        m = jnp.maximum(m, logits[w])
    e = [jnp.exp2((l - m) * (scale * LOG2E)) for l in logits]
    den = e[0]
    for w in range(1, WIN):
        den = den + e[w]
    inv = 1.0 / den
    p = [x * inv for x in e]
    for g in range(NG):
        acc = p[0] * window(2, g, 0)
        for w in range(1, WIN):
            acc = acc + p[w] * window(2, g, w)
        o_s[pl.ds(r, AR), g * 128:(g + 1) * 128] = acc.astype(BF16)


def _kernel(x_hbm, c_hbm, wqkv_hbm, wo_hbm, wg_hbm, wu_hbm, wd_hbm, wmod_hbm, out_hbm,
            x_s, c_s, wmod_s, wqkv_s, wo_raw, wo_s, wg_s, wu_s, wd_s, mod_s,
            qkv0_s, qkv_s, h_s, h1_s, o_s, x1_s, h2_s, act_s, out_s, sems, qsems, xsems, osems):
    t = pl.program_id(0)
    first = t == 0

    def mod_copy(i):
        return pltpu.make_async_copy(wmod_hbm.at[:, pl.ds(pl.multiple_of(i * D, D), D)], wmod_s.at[i], sems.at[i])

    def qkv_copy(p):
        rs = pl.ds(pl.multiple_of((p % QP) * (D // QP), D // QP), D // QP)
        return pltpu.make_async_copy(wqkv_hbm.at[rs, pl.ds(pl.multiple_of((p // QP) * D, D), D)],
                                     wqkv_s.at[p // QP, rs], qsems.at[p])

    def x_copy(i):
        return pltpu.make_async_copy(x_hbm.at[pl.ds(pl.multiple_of(i * TM, TM), TM)], x_s.at[i], xsems.at[i])

    def c_copy():
        return pltpu.make_async_copy(c_hbm, c_s, sems.at[6])

    def wo_copy():
        return pltpu.make_async_copy(wo_hbm, wo_raw, sems.at[9])

    def gate_copy(f):
        return pltpu.make_async_copy(wg_hbm.at[:, pl.ds(pl.multiple_of(f * FC, FC), FC)], wg_s.at[f], sems.at[10 + f])

    def up_copy(f):
        return pltpu.make_async_copy(wu_hbm.at[:, pl.ds(pl.multiple_of(f * FC, FC), FC)], wu_s.at[f], sems.at[10 + NF + f])

    def down_copy(n):
        return pltpu.make_async_copy(wd_hbm.at[:, pl.ds(pl.multiple_of(n * NC, NC), NC)], wd_s.at[n], sems.at[10 + 2 * NF + n])

    def out_copy(tile, n):
        rows = pl.ds(pl.multiple_of(tile * TM, TM), TM)
        return pltpu.make_async_copy(
            out_s.at[n], out_hbm.at[rows, pl.ds(pl.multiple_of(n * NC, NC), NC)], osems.at[n])

    def compute_mod(i, cs=slice(None)):
        cc = c_s[...].astype(F32)
        sc = jnp.broadcast_to(cc * jax.nn.sigmoid(cc), (16, D)).astype(BF16)
        mod_s[i, :, cs] = jnp.dot(sc, wmod_s[i, :, cs], preferred_element_type=F32)[0:8]

    def mod(i):
        return mod_s[i, 0:1, :]

    def modulated_ln(x, shift, scale):
        return (_layernorm(x) * (1.0 + mod(scale)) + mod(shift)).astype(BF16)

    def norm1(tile, dst, rs):
        dst[rs, :] = modulated_ln(x_s[tile, rs, :].astype(F32), 0, 1)

    def norm2(slot, rs):
        h2_s[rs, :] = modulated_ln(x1_s[slot, rs, :], 3, 4)

    def row_loop(rows, fn):
        def body(i, carry):
            fn(pl.ds(pl.multiple_of(i * rows, rows), rows))
            return carry

        lax.fori_loop(0, TM // rows, body, 0)

    def part(i, n):
        rows = -(-TM // (n * 16)) * 16
        return pl.ds(pl.multiple_of(jnp.minimum(i * rows, TM - rows), 16), rows)

    def attention_part(src, s0, i, n):
        per = -(-(TM // AR) // n)
        for b in range(per):
            blk = jnp.minimum(i * per + b, TM // AR - 1)
            _attention_block(s0, pl.multiple_of(blk * AR, AR), src, o_s, src is qkv0_s)

    def qkv_loop(src, dst, s0, pieces, copies, ride_along):
        def body(i, carry):
            copies(i)
            y = None
            for k in range(pieces):
                ks = slice(k * (D // pieces), (k + 1) * (D // pieces))
                yk = jnp.dot(src[:, ks], wqkv_s[i, ks, :], preferred_element_type=F32)
                y = yk if k == 0 else y + yk
                ride_along(i, k)
            rs = pl.ds(pl.multiple_of(HALO + s0, 8), TM)
            for g in range(NG):
                dst[i, g, rs, :] = y[:, g * 128:(g + 1) * 128]
            return carry

        lax.fori_loop(0, 3, body, 0)

    @pl.when(first)
    def _():
        for p in range(QP):
            qkv_copy(p).start()
        c_copy().start()
        qkv0_s[1:3, :, 0:HALO, :] = jnp.zeros((2, NG, HALO, 128), F32)

        def perm_body(p, carry):
            qkv_copy(p).wait()
            pl.when(p == 0)(mod_copy(0).start)
            pl.when(p == 2)(x_copy(0).start)
            pl.when(p == 3)(mod_copy(1).start)
            rows = D // QP
            _permute_columns(wqkv_s.at[0], pl.ds(pl.multiple_of(p * rows, rows), rows), True)
            return carry

        lax.fori_loop(0, QP, perm_body, 0)
        c_copy().wait()

        def mod_body(i, carry):
            mod_copy(i).wait()

            @pl.when(i == 1)
            def _():
                for p in range(QP, 2 * QP):
                    qkv_copy(p).start()

            compute_mod(i)
            return carry

        lax.fori_loop(0, 2, mod_body, 0)
        x_copy(0).wait()
        row_loop(128, lambda rs: norm1(0, h_s, rs))

        def copies_0(i):
            @pl.when(i == 0)
            def _():
                x_copy(1).start()
                for p in range(2 * QP, 3 * QP):
                    qkv_copy(p).start()

            @pl.when(i == 1)
            def _():
                x_copy(1).wait()
                wo_copy().start()

            for j in range(2):
                pl.when(i > 0)(mod_copy(2 * jnp.maximum(i, 1) + j).start)

            @pl.when(i < 2)
            def _():
                for p in range(QP):
                    qkv_copy((i + 1) * QP + p).wait()

        def ride_permute(i, k):
            _permute_columns(wqkv_s.at[i + 1], pl.ds(k * (D // KP), D // KP), False)
            norm1(jnp.minimum(i, 1), h1_s, part((jnp.maximum(i, 1) - 1) * KP + k, 2 * KP))

        qkv_loop(h_s, qkv0_s, 0, KP, copies_0, ride_permute)
        qkv_s[1:3, :, 0:HALO, :] = qkv0_s[1:3, :, TM:TM + HALO, :]
        wo_copy().wait()

        def copies_1(i):
            @pl.when(i == 0)
            def _():
                for j in range(2, NT):
                    x_copy(j).start()

            gate_copy(i).start()
            up_copy(i).start()

        def ride_attention(i, k):
            attention_part(qkv0_s, 0, i, 3)
            for j in range(3):
                _permute_rows(wo_raw, wo_s, jnp.minimum(3 * i + j, 7))

        qkv_loop(h1_s, qkv_s, 0, 1, copies_1, ride_attention)
        gate_copy(NF - 1).start()
        up_copy(NF - 1).start()
        for n in range(D // NC):
            down_copy(n).start()

        def mod_rest(i, carry):
            mod_copy(i).wait()
            compute_mod(i)
            return carry

        lax.fori_loop(2, 5, mod_rest, 0)

    @pl.when(t > 0)
    def _():
        pl.when(t + 1 < NT)(lambda: x_copy(t + 1).wait())

        def gate_up(f, carry):
            @pl.when(t == 1)
            def _():
                gate_copy(f).wait()
                up_copy(f).wait()

            norm1(jnp.minimum(t + 1, NT - 1), h_s, part(f, NF))
            attention_part(qkv_s, (jnp.minimum(t, NT - 1) - 1) * TM, f, NF)
            h2 = h2_s[...]
            g = jnp.dot(h2, wg_s[f], preferred_element_type=F32)
            u = jnp.dot(h2, wu_s[f], preferred_element_type=F32)
            hg = 0.5 * g
            act_s[f] = ((hg + hg * jnp.tanh(hg)) * u).astype(BF16)
            return carry

        lax.fori_loop(0, NF, gate_up, 0)

    @pl.when(t < NT)
    def _():
        a = jnp.dot(o_s[...], wo_s[...], preferred_element_type=F32)
        x1_s[t % 2] = x_s[t].astype(F32) + mod(2) * a

    @pl.when(first)
    def _():
        mod_copy(5).wait()

        def body(i, carry):
            norm2(0, part(i, 4))
            compute_mod(5, pl.ds(pl.multiple_of(i * (D // 4), D // 4), D // 4))
            return carry

        lax.fori_loop(0, 4, body, 0)

    @pl.when(t > 0)
    def _():
        def down(n, carry):
            @pl.when(t == 1)
            def _():
                down_copy(n).wait()

            pl.when(t > 1)(lambda: out_copy(t - 2, n).wait())
            norm2(jnp.minimum(t, NT - 1) % 2, part(n, D // NC))
            y = None
            for f in range(NF):
                yf = jnp.dot(act_s[f], wd_s[n, f * FC:(f + 1) * FC, :], preferred_element_type=F32)
                y = yf if f == 0 else y + yf
            cs = pl.ds(pl.multiple_of(n * NC, NC), NC)
            out_s[n] = (x1_s[1 - t % 2, :, cs] + mod_s[5, 0:1, cs] * y).astype(out_s.dtype)
            out_copy(t - 1, n).start()
            return carry

        lax.fori_loop(0, D // NC, down, 0)

    @pl.when(jnp.logical_and(t > 0, t + 1 < NT))
    def _():
        qkv_loop(h_s, qkv_s, t * TM, 1, lambda i: None, lambda i, k: None)

    @pl.when(t == NT)
    def _():
        for n in range(D // NC):
            out_copy(NT - 1, n).wait()


@jax.jit
def pallas_adaLN_cond__sliding_local_dilated__swiglu_ffn__prompt_kernel(
    A_x: jax.Array,
    A_wqkv: jax.Array,
    A_wo: jax.Array,
    B_x: jax.Array,
    B_w_gate: jax.Array,
    B_w_up: jax.Array,
    B_w_down: jax.Array,
    c: jax.Array,
    w_mod: jax.Array,
):
    del B_x
    hbm = pl.BlockSpec(memory_space=pl.ANY)
    out = pl.pallas_call(
        _kernel,
        grid=(NT + 1,),
        in_specs=[hbm] * 8,
        out_specs=hbm,
        out_shape=jax.ShapeDtypeStruct((S, D), A_x.dtype),
        scratch_shapes=[
            pltpu.VMEM((NT, TM, D), BF16),
            pltpu.VMEM((1, D), BF16),
            pltpu.VMEM((6, D, D), BF16),
            pltpu.VMEM((4, D, D), BF16),
            pltpu.VMEM((D, D), BF16),
            pltpu.VMEM((D, D), BF16),
            pltpu.VMEM((NF, D, FC), BF16),
            pltpu.VMEM((NF, D, FC), BF16),
            pltpu.VMEM((D // NC, F, NC), BF16),
            pltpu.VMEM((6, 8, D), F32),
            pltpu.VMEM((3, NG, HALO + TM, 128), F32),
            pltpu.VMEM((3, NG, HALO + S - TM, 128), F32),
            pltpu.VMEM((TM, D), BF16),
            pltpu.VMEM((TM, D), BF16),
            pltpu.VMEM((TM, D), BF16),
            pltpu.VMEM((2, TM, D), F32),
            pltpu.VMEM((TM, D), BF16),
            pltpu.VMEM((NF, TM, FC), BF16),
            pltpu.VMEM((D // NC, TM, NC), A_x.dtype),
            pltpu.SemaphoreType.DMA((10 + 2 * NF + D // NC,)),
            pltpu.SemaphoreType.DMA((3 * QP,)),
            pltpu.SemaphoreType.DMA((NT,)),
            pltpu.SemaphoreType.DMA((D // NC,)),
        ],
        compiler_params=pltpu.CompilerParams(
            dimension_semantics=("arbitrary",),
            flags={'XLA_TPU_EVENLY_DISTRIBUTE_CRITICAL_NODES': True},
            vmem_limit_bytes=112 * 1024 * 1024,
        ),
    )(A_x.reshape(S, D), c, A_wqkv, A_wo, B_w_gate, B_w_up, B_w_down, w_mod)
    return out.reshape(A_x.shape)
```

```python
import jax
import jax.numpy as jnp
from jax import lax
from jax.experimental import pallas as pl
from jax.experimental.pallas import tpu as pltpu

S, D, F = 2048, 1024, 3584
H, DH, WIN, DIL = 32, 32, 8, 2
TM = 512
NT = S // TM
FC = 896
NF = F // FC
NC = 256
DU = 2
HALO = 16
AR = 16
KP = 8
QP = 4
NG = D // 128
EPS = 1e-5
LOG2E = 1.4426950408889634
F32, BF16 = jnp.float32, jnp.bfloat16


def _layernorm(x):
    m = jnp.mean(x, axis=-1, keepdims=True)
    xc = x - m
    v = jnp.mean(xc * xc, axis=-1, keepdims=True)
    return xc * lax.rsqrt(v + EPS)


def _swap_group_and_field(xs, field, roll):
    xs = [roll(xs[-g % 8], -g % 8) for g in range(8)]
    for b in (1, 2, 4):
        bit = (field & b) != 0
        xs = [jnp.where(bit, xs[(g - b) % 8], xs[g]) for g in range(8)]
    return [roll(x, -g) for g, x in enumerate(xs)]


def _permute_columns(w_ref, rs, on_mxu):
    shift = (lax.broadcasted_iota(jnp.int32, (128, 128), 1)
             - lax.broadcasted_iota(jnp.int32, (128, 128), 0)) & 127

    def roll(x, n):
        if n == 0:
            return x
        if not on_mxu:
            return pltpu.roll(x, 2 * n % 128, 1)
        rot = (shift == 2 * n % 128).astype(F32).astype(BF16)
        y = jnp.dot(pltpu.bitcast(x, BF16), rot, preferred_element_type=F32)
        return pltpu.bitcast(y.astype(BF16), jnp.uint32)

    cols = [pltpu.bitcast(w_ref[rs, g * 128:(g + 1) * 128], jnp.uint32) for g in range(NG)]
    field = lax.broadcasted_iota(jnp.int32, cols[0].shape, 1) >> 1
    for g, x in enumerate(_swap_group_and_field(cols, field, roll)):
        w_ref[rs, g * 128:(g + 1) * 128] = pltpu.bitcast(x, BF16)


def _permute_rows(src_ref, dst_ref, m):
    rows = [pl.ds(pl.multiple_of(c * 128 + m * 16, 16), 16) for c in range(8)]
    field = lax.broadcasted_iota(jnp.int32, (8, 128), 0)
    for g in range(NG):
        cs = slice(g * 128, (g + 1) * 128)
        xs = [pltpu.bitcast(src_ref[r, cs], jnp.uint32) for r in rows]
        xs = _swap_group_and_field(xs, field, lambda x, n: pltpu.roll(x, n % 8, 0) if n else x)
        for r, x in zip(rows, xs):
            dst_ref[r, cs] = pltpu.bitcast(x, BF16)


def _attention_block(s0, r, qkv_s, o_s, masked):
    scale = DH ** -0.5
    lane = lax.broadcasted_iota(jnp.int32, (AR, 128), 1)

    def window(which, g, w):
        return qkv_s[which, g, pl.ds(s0 + r + (HALO - DIL * w), AR), :]

    q = [window(0, g, 0) for g in range(NG)]
    logits = []
    for w in range(WIN):
        acc = q[0] * window(1, 0, w)
        for g in range(1, NG):
            acc = acc + q[g] * window(1, g, w)
        logits.append(acc)
    for sh in (1, 16):
        low = (lane & sh) == 0
        logits = [x + jnp.where(low, pltpu.roll(x, 128 - sh, 1), pltpu.roll(x, sh, 1)) for x in logits]
    if masked:
        pos = lax.broadcasted_iota(jnp.int32, (AR, 128), 0) + r
        logits = [jnp.where(pos >= DIL * w, x, -1e9 / scale) if w else x for w, x in enumerate(logits)]
    m = logits[0]
    for w in range(1, WIN):
        m = jnp.maximum(m, logits[w])
    e = [jnp.exp2((l - m) * (scale * LOG2E)) for l in logits]
    den = e[0]
    for w in range(1, WIN):
        den = den + e[w]
    inv = 1.0 / den
    p = [x * inv for x in e]
    for g in range(NG):
        acc = p[0] * window(2, g, 0)
        for w in range(1, WIN):
            acc = acc + p[w] * window(2, g, w)
        o_s[pl.ds(r, AR), g * 128:(g + 1) * 128] = acc.astype(BF16)


def _kernel(x_hbm, c_hbm, wqkv_hbm, wo_hbm, wg_hbm, wu_hbm, wd_hbm, wmod_hbm, out_hbm,
            x_s, c_s, wmod_s, wqkv_s, wo_raw, wo_s, wg_s, wu_s, wd_s, mod_s,
            qkv0_s, qkv_s, h_s, h1_s, o_s, x1_s, h2_s, act_s, out_s, sems, qsems, xsems, osems):
    t = pl.program_id(0)
    first = t == 0

    def mod_copy(i):
        return pltpu.make_async_copy(wmod_hbm.at[:, pl.ds(pl.multiple_of(i * D, D), D)], wmod_s.at[i], sems.at[i])

    def qkv_copy(p):
        rs = pl.ds(pl.multiple_of((p % QP) * (D // QP), D // QP), D // QP)
        return pltpu.make_async_copy(wqkv_hbm.at[rs, pl.ds(pl.multiple_of((p // QP) * D, D), D)],
                                     wqkv_s.at[p // QP, rs], qsems.at[p])

    def x_copy(i):
        return pltpu.make_async_copy(x_hbm.at[pl.ds(pl.multiple_of(i * TM, TM), TM)], x_s.at[i], xsems.at[i])

    def c_copy():
        return pltpu.make_async_copy(c_hbm, c_s, sems.at[6])

    def wo_copy():
        return pltpu.make_async_copy(wo_hbm, wo_raw, sems.at[9])

    def gate_copy(f):
        return pltpu.make_async_copy(wg_hbm.at[:, pl.ds(pl.multiple_of(f * FC, FC), FC)], wg_s.at[f], sems.at[10 + f])

    def up_copy(f):
        return pltpu.make_async_copy(wu_hbm.at[:, pl.ds(pl.multiple_of(f * FC, FC), FC)], wu_s.at[f], sems.at[10 + NF + f])

    def down_copy(n):
        return pltpu.make_async_copy(wd_hbm.at[:, pl.ds(pl.multiple_of(n * NC, NC), NC)], wd_s.at[n], sems.at[10 + 2 * NF + n])

    def out_copy(tile, n):
        rows = pl.ds(pl.multiple_of(tile * TM, TM), TM)
        return pltpu.make_async_copy(
            out_s.at[n], out_hbm.at[rows, pl.ds(pl.multiple_of(n * NC, NC), NC)], osems.at[n])

    def compute_mod(i, cs=slice(None)):
        cc = c_s[...].astype(F32)
        sc = jnp.broadcast_to(cc * jax.nn.sigmoid(cc), (16, D)).astype(BF16)
        mod_s[i, :, cs] = jnp.dot(sc, wmod_s[i, :, cs], preferred_element_type=F32)[0:8]

    def mod(i):
        return mod_s[i, 0:1, :]

    def modulated_ln(x, shift, scale):
        return (_layernorm(x) * (1.0 + mod(scale)) + mod(shift)).astype(BF16)

    def norm1(tile, dst, rs):
        dst[rs, :] = modulated_ln(x_s[tile, rs, :].astype(F32), 0, 1)

    def norm2(slot, rs):
        h2_s[rs, :] = modulated_ln(x1_s[slot, rs, :], 3, 4)

    def row_loop(rows, fn):
        def body(i, carry):
            fn(pl.ds(pl.multiple_of(i * rows, rows), rows))
            return carry

        lax.fori_loop(0, TM // rows, body, 0)

    def part(i, n):
        rows = -(-TM // (n * 16)) * 16
        return pl.ds(pl.multiple_of(jnp.minimum(i * rows, TM - rows), 16), rows)

    def attention_part(src, s0, i, n):
        per = -(-(TM // AR) // n)
        for b in range(per):
            blk = jnp.minimum(i * per + b, TM // AR - 1)
            _attention_block(s0, pl.multiple_of(blk * AR, AR), src, o_s, src is qkv0_s)

    def qkv_loop(src, dst, s0, pieces, copies, ride_along):
        def body(i, carry):
            copies(i)
            y = None
            for k in range(pieces):
                ks = slice(k * (D // pieces), (k + 1) * (D // pieces))
                yk = jnp.dot(src[:, ks], wqkv_s[i, ks, :], preferred_element_type=F32)
                y = yk if k == 0 else y + yk
                ride_along(i, k)
            rs = pl.ds(pl.multiple_of(HALO + s0, 8), TM)
            for g in range(NG):
                dst[i, g, rs, :] = y[:, g * 128:(g + 1) * 128]
            return carry

        lax.fori_loop(0, 3, body, 0)

    @pl.when(first)
    def _():
        for p in range(QP):
            qkv_copy(p).start()
        c_copy().start()
        qkv0_s[1:3, :, 0:HALO, :] = jnp.zeros((2, NG, HALO, 128), F32)

        def perm_body(p, carry):
            qkv_copy(p).wait()
            pl.when(p == 0)(mod_copy(0).start)
            pl.when(p == 2)(x_copy(0).start)
            pl.when(p == 3)(mod_copy(1).start)
            rows = D // QP
            _permute_columns(wqkv_s.at[0], pl.ds(pl.multiple_of(p * rows, rows), rows), True)
            return carry

        lax.fori_loop(0, QP, perm_body, 0)
        c_copy().wait()

        def mod_body(i, carry):
            mod_copy(i).wait()

            @pl.when(i == 1)
            def _():
                for p in range(QP, 2 * QP):
                    qkv_copy(p).start()

            compute_mod(i)
            return carry

        lax.fori_loop(0, 2, mod_body, 0)
        x_copy(0).wait()
        row_loop(128, lambda rs: norm1(0, h_s, rs))

        def copies_0(i):
            @pl.when(i == 0)
            def _():
                x_copy(1).start()
                for p in range(2 * QP, 3 * QP):
                    qkv_copy(p).start()

            @pl.when(i == 1)
            def _():
                x_copy(1).wait()
                wo_copy().start()

            for j in range(2):
                pl.when(i > 0)(mod_copy(2 * jnp.maximum(i, 1) + j).start)

            @pl.when(i < 2)
            def _():
                for p in range(QP):
                    qkv_copy((i + 1) * QP + p).wait()

        def ride_permute(i, k):
            _permute_columns(wqkv_s.at[i + 1], pl.ds(k * (D // KP), D // KP), False)
            norm1(jnp.minimum(i, 1), h1_s, part((jnp.maximum(i, 1) - 1) * KP + k, 2 * KP))

        qkv_loop(h_s, qkv0_s, 0, KP, copies_0, ride_permute)
        qkv_s[1:3, :, 0:HALO, :] = qkv0_s[1:3, :, TM:TM + HALO, :]
        wo_copy().wait()

        def copies_1(i):
            @pl.when(i == 0)
            def _():
                for j in range(2, NT):
                    x_copy(j).start()

            gate_copy(i).start()
            up_copy(i).start()

        def ride_attention(i, k):
            attention_part(qkv0_s, 0, i, 3)
            for j in range(3):
                _permute_rows(wo_raw, wo_s, jnp.minimum(3 * i + j, 7))

        qkv_loop(h1_s, qkv_s, 0, 1, copies_1, ride_attention)
        gate_copy(NF - 1).start()
        up_copy(NF - 1).start()
        for n in range(D // NC):
            down_copy(n).start()

        def mod_rest(i, carry):
            mod_copy(i).wait()
            compute_mod(i)
            return carry

        lax.fori_loop(2, 5, mod_rest, 0)

    @pl.when(t > 0)
    def _():
        pl.when(t + 1 < NT)(lambda: x_copy(t + 1).wait())

        def gate_up(f, carry):
            @pl.when(t == 1)
            def _():
                gate_copy(f).wait()
                up_copy(f).wait()

            norm1(jnp.minimum(t + 1, NT - 1), h_s, part(f, NF))
            attention_part(qkv_s, (jnp.minimum(t, NT - 1) - 1) * TM, f, NF)
            h2 = h2_s[...]
            g = jnp.dot(h2, wg_s[f], preferred_element_type=F32)
            u = jnp.dot(h2, wu_s[f], preferred_element_type=F32)
            hg = 0.5 * g
            act_s[f] = ((hg + hg * jnp.tanh(hg)) * u).astype(BF16)
            return carry

        lax.fori_loop(0, NF, gate_up, 0)

    @pl.when(t < NT)
    def _():
        a = jnp.dot(o_s[...], wo_s[...], preferred_element_type=F32)
        x1_s[t % 2] = x_s[t].astype(F32) + mod(2) * a

    @pl.when(first)
    def _():
        mod_copy(5).wait()

        def body(i, carry):
            norm2(0, part(i, 4))
            compute_mod(5, pl.ds(pl.multiple_of(i * (D // 4), D // 4), D // 4))
            return carry

        lax.fori_loop(0, 4, body, 0)

    @pl.when(t > 0)
    def _():
        def down(i, carry):
            chunks = [DU * i + j for j in range(DU)]

            @pl.when(t == 1)
            def _():
                for n in chunks:
                    down_copy(n).wait()

            @pl.when(t > 1)
            def _():
                for n in chunks:
                    out_copy(t - 2, n).wait()

            norm2(jnp.minimum(t, NT - 1) % 2, part(i, D // NC // DU))
            for n in chunks:
                y = None
                for f in range(NF):
                    yf = jnp.dot(act_s[f], wd_s[n, f * FC:(f + 1) * FC, :], preferred_element_type=F32)
                    y = yf if f == 0 else y + yf
                cs = pl.ds(pl.multiple_of(n * NC, NC), NC)
                out_s[n] = (x1_s[1 - t % 2, :, cs] + mod_s[5, 0:1, cs] * y).astype(out_s.dtype)
                out_copy(t - 1, n).start()
            return carry

        lax.fori_loop(0, D // NC // DU, down, 0)

    @pl.when(jnp.logical_and(t > 0, t + 1 < NT))
    def _():
        qkv_loop(h_s, qkv_s, t * TM, 1, lambda i: None, lambda i, k: None)

    @pl.when(t == NT)
    def _():
        for n in range(D // NC):
            out_copy(NT - 1, n).wait()


@jax.jit
def pallas_adaLN_cond__sliding_local_dilated__swiglu_ffn__prompt_kernel(
    A_x: jax.Array,
    A_wqkv: jax.Array,
    A_wo: jax.Array,
    B_x: jax.Array,
    B_w_gate: jax.Array,
    B_w_up: jax.Array,
    B_w_down: jax.Array,
    c: jax.Array,
    w_mod: jax.Array,
):
    del B_x
    hbm = pl.BlockSpec(memory_space=pl.ANY)
    out = pl.pallas_call(
        _kernel,
        grid=(NT + 1,),
        in_specs=[hbm] * 8,
        out_specs=hbm,
        out_shape=jax.ShapeDtypeStruct((S, D), A_x.dtype),
        scratch_shapes=[
            pltpu.VMEM((NT, TM, D), BF16),
            pltpu.VMEM((1, D), BF16),
            pltpu.VMEM((6, D, D), BF16),
            pltpu.VMEM((4, D, D), BF16),
            pltpu.VMEM((D, D), BF16),
            pltpu.VMEM((D, D), BF16),
            pltpu.VMEM((NF, D, FC), BF16),
            pltpu.VMEM((NF, D, FC), BF16),
            pltpu.VMEM((D // NC, F, NC), BF16),
            pltpu.VMEM((6, 8, D), F32),
            pltpu.VMEM((3, NG, HALO + TM, 128), F32),
            pltpu.VMEM((3, NG, HALO + S - TM, 128), F32),
            pltpu.VMEM((TM, D), BF16),
            pltpu.VMEM((TM, D), BF16),
            pltpu.VMEM((TM, D), BF16),
            pltpu.VMEM((2, TM, D), F32),
            pltpu.VMEM((TM, D), BF16),
            pltpu.VMEM((NF, TM, FC), BF16),
            pltpu.VMEM((D // NC, TM, NC), A_x.dtype),
            pltpu.SemaphoreType.DMA((10 + 2 * NF + D // NC,)),
            pltpu.SemaphoreType.DMA((3 * QP,)),
            pltpu.SemaphoreType.DMA((NT,)),
            pltpu.SemaphoreType.DMA((D // NC,)),
        ],
        compiler_params=pltpu.CompilerParams(
            dimension_semantics=("arbitrary",),
            flags={'XLA_TPU_EVENLY_DISTRIBUTE_CRITICAL_NODES': True},
            vmem_limit_bytes=112 * 1024 * 1024,
        ),
    )(A_x.reshape(S, D), c, A_wqkv, A_wo, B_w_gate, B_w_up, B_w_down, w_mod)
    return out.reshape(A_x.shape)
```

```python
import jax
import jax.numpy as jnp
from jax import lax
from jax.experimental import pallas as pl
from jax.experimental.pallas import tpu as pltpu

S, D, F = 2048, 1024, 3584
H, DH, WIN, DIL = 32, 32, 8, 2
TM = 512
NT = S // TM
FC = 896
NF = F // FC
NC = 256
DU = 2
HALO = 16
AR = 16
KP = 8
QP = 4
NG = D // 128
EPS = 1e-5
LOG2E = 1.4426950408889634
F32, BF16 = jnp.float32, jnp.bfloat16


def _layernorm(x):
    m = jnp.mean(x, axis=-1, keepdims=True)
    xc = x - m
    v = jnp.mean(xc * xc, axis=-1, keepdims=True)
    return xc * lax.rsqrt(v + EPS)


def _swap_group_and_field(xs, field, roll):
    xs = [roll(xs[-g % 8], -g % 8) for g in range(8)]
    for b in (1, 2, 4):
        bit = (field & b) != 0
        xs = [jnp.where(bit, xs[(g - b) % 8], xs[g]) for g in range(8)]
    return [roll(x, -g) for g, x in enumerate(xs)]


def _permute_columns(w_ref, rs, on_mxu):
    shift = (lax.broadcasted_iota(jnp.int32, (128, 128), 1)
             - lax.broadcasted_iota(jnp.int32, (128, 128), 0)) & 127

    def roll(x, n):
        if n == 0:
            return x
        if not on_mxu:
            return pltpu.roll(x, 2 * n % 128, 1)
        rot = (shift == 2 * n % 128).astype(F32).astype(BF16)
        y = jnp.dot(pltpu.bitcast(x, BF16), rot, preferred_element_type=F32)
        return pltpu.bitcast(y.astype(BF16), jnp.uint32)

    cols = [pltpu.bitcast(w_ref[rs, g * 128:(g + 1) * 128], jnp.uint32) for g in range(NG)]
    field = lax.broadcasted_iota(jnp.int32, cols[0].shape, 1) >> 1
    for g, x in enumerate(_swap_group_and_field(cols, field, roll)):
        w_ref[rs, g * 128:(g + 1) * 128] = pltpu.bitcast(x, BF16)


def _permute_rows(src_ref, dst_ref, m):
    rows = [pl.ds(pl.multiple_of(c * 128 + m * 16, 16), 16) for c in range(8)]
    field = lax.broadcasted_iota(jnp.int32, (8, 128), 0)
    for g in range(NG):
        cs = slice(g * 128, (g + 1) * 128)
        xs = [pltpu.bitcast(src_ref[r, cs], jnp.uint32) for r in rows]
        xs = _swap_group_and_field(xs, field, lambda x, n: pltpu.roll(x, n % 8, 0) if n else x)
        for r, x in zip(rows, xs):
            dst_ref[r, cs] = pltpu.bitcast(x, BF16)


def _attention_block(s0, r, qkv_s, o_s, masked):
    scale = DH ** -0.5
    lane = lax.broadcasted_iota(jnp.int32, (AR, 128), 1)

    def window(which, g, w):
        return qkv_s[which, g, pl.ds(s0 + r + (HALO - DIL * w), AR), :]

    q = [window(0, g, 0) for g in range(NG)]
    logits = []
    for w in range(WIN):
        acc = q[0] * window(1, 0, w)
        for g in range(1, NG):
            acc = acc + q[g] * window(1, g, w)
        logits.append(acc)
    for sh in (1, 16):
        low = (lane & sh) == 0
        logits = [x + jnp.where(low, pltpu.roll(x, 128 - sh, 1), pltpu.roll(x, sh, 1)) for x in logits]
    if masked:
        pos = lax.broadcasted_iota(jnp.int32, (AR, 128), 0) + r
        logits = [jnp.where(pos >= DIL * w, x, -1e9 / scale) if w else x for w, x in enumerate(logits)]
    m = logits[0]
    for w in range(1, WIN):
        m = jnp.maximum(m, logits[w])
    e = [jnp.exp2((l - m) * (scale * LOG2E)) for l in logits]
    den = e[0]
    for w in range(1, WIN):
        den = den + e[w]
    inv = 1.0 / den
    p = [x * inv for x in e]
    for g in range(NG):
        acc = p[0] * window(2, g, 0)
        for w in range(1, WIN):
            acc = acc + p[w] * window(2, g, w)
        o_s[pl.ds(r, AR), g * 128:(g + 1) * 128] = acc.astype(BF16)


def _kernel(x_hbm, c_hbm, wqkv_hbm, wo_hbm, wg_hbm, wu_hbm, wd_hbm, wmod_hbm, out_hbm,
            x_s, c_s, wmod_s, wqkv_s, wo_raw, wo_s, wg_s, wu_s, wd_s, mod_s,
            qkv0_s, qkv_s, h_s, h1_s, o_s, x1_s, h2_s, act_s, out_s, sems, qsems, xsems, osems):
    t = pl.program_id(0)
    first = t == 0

    def mod_copy(i):
        return pltpu.make_async_copy(wmod_hbm.at[:, pl.ds(pl.multiple_of(i * D, D), D)], wmod_s.at[i], sems.at[i])

    def qkv_copy(p):
        rs = pl.ds(pl.multiple_of((p % QP) * (D // QP), D // QP), D // QP)
        return pltpu.make_async_copy(wqkv_hbm.at[rs, pl.ds(pl.multiple_of((p // QP) * D, D), D)],
                                     wqkv_s.at[p // QP, rs], qsems.at[p])

    def x_copy(i):
        return pltpu.make_async_copy(x_hbm.at[pl.ds(pl.multiple_of(i * TM, TM), TM)], x_s.at[i], xsems.at[i])

    def c_copy():
        return pltpu.make_async_copy(c_hbm, c_s, sems.at[6])

    def wo_copy():
        return pltpu.make_async_copy(wo_hbm, wo_raw, sems.at[9])

    def gate_copy(f):
        return pltpu.make_async_copy(wg_hbm.at[:, pl.ds(pl.multiple_of(f * FC, FC), FC)], wg_s.at[f], sems.at[10 + f])

    def up_copy(f):
        return pltpu.make_async_copy(wu_hbm.at[:, pl.ds(pl.multiple_of(f * FC, FC), FC)], wu_s.at[f], sems.at[10 + NF + f])

    def down_copy(n):
        return pltpu.make_async_copy(wd_hbm.at[:, pl.ds(pl.multiple_of(n * NC, NC), NC)], wd_s.at[n], sems.at[10 + 2 * NF + n])

    def out_copy(tile, n):
        rows = pl.ds(pl.multiple_of(tile * TM, TM), TM)
        return pltpu.make_async_copy(
            out_s.at[n], out_hbm.at[rows, pl.ds(pl.multiple_of(n * NC, NC), NC)], osems.at[n])

    def compute_mod(i, cs=slice(None)):
        cc = c_s[...].astype(F32)
        sc = jnp.broadcast_to(cc * jax.nn.sigmoid(cc), (16, D)).astype(BF16)
        mod_s[i, :, cs] = jnp.dot(sc, wmod_s[i, :, cs], preferred_element_type=F32)[0:8]

    def mod(i):
        return mod_s[i, 0:1, :]

    def modulated_ln(x, shift, scale):
        return (_layernorm(x) * (1.0 + mod(scale)) + mod(shift)).astype(BF16)

    def norm1(tile, dst, rs):
        dst[rs, :] = modulated_ln(x_s[tile, rs, :].astype(F32), 0, 1)

    def norm2(slot, rs):
        h2_s[rs, :] = modulated_ln(x1_s[slot, rs, :], 3, 4)

    def row_loop(rows, fn):
        def body(i, carry):
            fn(pl.ds(pl.multiple_of(i * rows, rows), rows))
            return carry

        lax.fori_loop(0, TM // rows, body, 0)

    def part(i, n):
        rows = -(-TM // (n * 16)) * 16
        return pl.ds(pl.multiple_of(jnp.minimum(i * rows, TM - rows), 16), rows)

    def attention_part(src, s0, i, n):
        per = -(-(TM // AR) // n)
        for b in range(per):
            blk = jnp.minimum(i * per + b, TM // AR - 1)
            _attention_block(s0, pl.multiple_of(blk * AR, AR), src, o_s, src is qkv0_s)

    def qkv_loop(src, dst, s0, pieces, copies, ride_along):
        def body(i, carry):
            copies(i)
            y = None
            for k in range(pieces):
                ks = slice(k * (D // pieces), (k + 1) * (D // pieces))
                yk = jnp.dot(src[:, ks], wqkv_s[i, ks, :], preferred_element_type=F32)
                y = yk if k == 0 else y + yk
                ride_along(i, k)
            rs = pl.ds(pl.multiple_of(HALO + s0, 8), TM)
            for g in range(NG):
                dst[i, g, rs, :] = y[:, g * 128:(g + 1) * 128]
            return carry

        lax.fori_loop(0, 3, body, 0)

    @pl.when(first)
    def _():
        for p in range(QP // 2):
            qkv_copy(p).start()
        mod_copy(0).start()
        c_copy().start()
        qkv0_s[1:3, :, 0:HALO, :] = jnp.zeros((2, NG, HALO, 128), F32)

        def perm_body(p, carry):
            qkv_copy(p).wait()

            @pl.when(p == 0)
            def _():
                for later in range(QP // 2, QP):
                    qkv_copy(later).start()

            @pl.when(p == QP // 2)
            def _():
                x_copy(0).start()
                mod_copy(1).start()

            rows = D // QP
            _permute_columns(wqkv_s.at[0], pl.ds(pl.multiple_of(p * rows, rows), rows), True)
            return carry

        lax.fori_loop(0, QP, perm_body, 0)
        c_copy().wait()

        def mod_body(i, carry):
            mod_copy(i).wait()

            pl.when(i == 0)(qkv_copy(QP).start)

            @pl.when(i == 1)
            def _():
                for p in range(QP + 1, 2 * QP):
                    qkv_copy(p).start()

            compute_mod(i)
            return carry

        lax.fori_loop(0, 2, mod_body, 0)
        x_copy(0).wait()
        row_loop(128, lambda rs: norm1(0, h_s, rs))

        def copies_0(i):
            @pl.when(i == 0)
            def _():
                x_copy(1).start()
                for p in range(2 * QP, 3 * QP):
                    qkv_copy(p).start()

            @pl.when(i == 1)
            def _():
                x_copy(1).wait()
                wo_copy().start()

            for j in range(2):
                pl.when(i > 0)(mod_copy(2 * jnp.maximum(i, 1) + j).start)

            @pl.when(i < 2)
            def _():
                for p in range(QP):
                    qkv_copy((i + 1) * QP + p).wait()

        def ride_permute(i, k):
            _permute_columns(wqkv_s.at[i + 1], pl.ds(k * (D // KP), D // KP), False)
            norm1(jnp.minimum(i, 1), h1_s, part((jnp.maximum(i, 1) - 1) * KP + k, 2 * KP))

        qkv_loop(h_s, qkv0_s, 0, KP, copies_0, ride_permute)
        qkv_s[1:3, :, 0:HALO, :] = qkv0_s[1:3, :, TM:TM + HALO, :]
        wo_copy().wait()

        def copies_1(i):
            @pl.when(i == 0)
            def _():
                for j in range(2, NT):
                    x_copy(j).start()

            gate_copy(i).start()
            up_copy(i).start()

        def ride_attention(i, k):
            attention_part(qkv0_s, 0, i, 3)
            for j in range(3):
                _permute_rows(wo_raw, wo_s, jnp.minimum(3 * i + j, 7))

        qkv_loop(h1_s, qkv_s, 0, 1, copies_1, ride_attention)
        gate_copy(NF - 1).start()
        up_copy(NF - 1).start()
        for n in range(D // NC):
            down_copy(n).start()

        def mod_rest(i, carry):
            mod_copy(i).wait()
            compute_mod(i)
            return carry

        lax.fori_loop(2, 5, mod_rest, 0)

    @pl.when(t > 0)
    def _():
        pl.when(t + 1 < NT)(lambda: x_copy(t + 1).wait())

        def gate_up(f, carry):
            @pl.when(t == 1)
            def _():
                gate_copy(f).wait()
                up_copy(f).wait()

            norm1(jnp.minimum(t + 1, NT - 1), h_s, part(f, NF))
            attention_part(qkv_s, (jnp.minimum(t, NT - 1) - 1) * TM, f, NF)
            h2 = h2_s[...]
            g = jnp.dot(h2, wg_s[f], preferred_element_type=F32)
            u = jnp.dot(h2, wu_s[f], preferred_element_type=F32)
            hg = 0.5 * g
            act_s[f] = ((hg + hg * jnp.tanh(hg)) * u).astype(BF16)
            return carry

        lax.fori_loop(0, NF, gate_up, 0)

    @pl.when(t < NT)
    def _():
        a = jnp.dot(o_s[...], wo_s[...], preferred_element_type=F32)
        x1_s[t % 2] = x_s[t].astype(F32) + mod(2) * a

    @pl.when(first)
    def _():
        mod_copy(5).wait()

        def body(i, carry):
            norm2(0, part(i, 4))
            compute_mod(5, pl.ds(pl.multiple_of(i * (D // 4), D // 4), D // 4))
            return carry

        lax.fori_loop(0, 4, body, 0)

    @pl.when(t > 0)
    def _():
        def down(i, carry):
            chunks = [DU * i + j for j in range(DU)]

            @pl.when(t == 1)
            def _():
                for n in chunks:
                    down_copy(n).wait()

            @pl.when(t > 1)
            def _():
                for n in chunks:
                    out_copy(t - 2, n).wait()

            norm2(jnp.minimum(t, NT - 1) % 2, part(i, D // NC // DU))
            for n in chunks:
                y = None
                for f in range(NF):
                    yf = jnp.dot(act_s[f], wd_s[n, f * FC:(f + 1) * FC, :], preferred_element_type=F32)
                    y = yf if f == 0 else y + yf
                cs = pl.ds(pl.multiple_of(n * NC, NC), NC)
                out_s[n] = (x1_s[1 - t % 2, :, cs] + mod_s[5, 0:1, cs] * y).astype(out_s.dtype)
                out_copy(t - 1, n).start()
            return carry

        lax.fori_loop(0, D // NC // DU, down, 0)

    @pl.when(jnp.logical_and(t > 0, t + 1 < NT))
    def _():
        qkv_loop(h_s, qkv_s, t * TM, 1, lambda i: None, lambda i, k: None)

    @pl.when(t == NT)
    def _():
        for n in range(D // NC):
            out_copy(NT - 1, n).wait()


@jax.jit
def pallas_adaLN_cond__sliding_local_dilated__swiglu_ffn__prompt_kernel(
    A_x: jax.Array,
    A_wqkv: jax.Array,
    A_wo: jax.Array,
    B_x: jax.Array,
    B_w_gate: jax.Array,
    B_w_up: jax.Array,
    B_w_down: jax.Array,
    c: jax.Array,
    w_mod: jax.Array,
):
    del B_x
    hbm = pl.BlockSpec(memory_space=pl.ANY)
    out = pl.pallas_call(
        _kernel,
        grid=(NT + 1,),
        in_specs=[hbm] * 8,
        out_specs=hbm,
        out_shape=jax.ShapeDtypeStruct((S, D), A_x.dtype),
        scratch_shapes=[
            pltpu.VMEM((NT, TM, D), BF16),
            pltpu.VMEM((1, D), BF16),
            pltpu.VMEM((6, D, D), BF16),
            pltpu.VMEM((4, D, D), BF16),
            pltpu.VMEM((D, D), BF16),
            pltpu.VMEM((D, D), BF16),
            pltpu.VMEM((NF, D, FC), BF16),
            pltpu.VMEM((NF, D, FC), BF16),
            pltpu.VMEM((D // NC, F, NC), BF16),
            pltpu.VMEM((6, 8, D), F32),
            pltpu.VMEM((3, NG, HALO + TM, 128), F32),
            pltpu.VMEM((3, NG, HALO + S - TM, 128), F32),
            pltpu.VMEM((TM, D), BF16),
            pltpu.VMEM((TM, D), BF16),
            pltpu.VMEM((TM, D), BF16),
            pltpu.VMEM((2, TM, D), F32),
            pltpu.VMEM((TM, D), BF16),
            pltpu.VMEM((NF, TM, FC), BF16),
            pltpu.VMEM((D // NC, TM, NC), A_x.dtype),
            pltpu.SemaphoreType.DMA((10 + 2 * NF + D // NC,)),
            pltpu.SemaphoreType.DMA((3 * QP,)),
            pltpu.SemaphoreType.DMA((NT,)),
            pltpu.SemaphoreType.DMA((D // NC,)),
        ],
        compiler_params=pltpu.CompilerParams(
            dimension_semantics=("arbitrary",),
            flags={'XLA_TPU_EVENLY_DISTRIBUTE_CRITICAL_NODES': True},
            vmem_limit_bytes=112 * 1024 * 1024,
        ),
    )(A_x.reshape(S, D), c, A_wqkv, A_wo, B_w_gate, B_w_up, B_w_down, w_mod)
    return out.reshape(A_x.shape)
```
